```python
import jax
import jax.numpy as jnp

def _softmax(x, axis=-1):
    return jax.nn.softmax(x, axis=axis)
def _gelu(x):
    return jax.nn.gelu(x, approximate=True)
def _silu(x):
    return jax.nn.silu(x)
def _sigmoid(x):
    return jax.nn.sigmoid(x)
def _layernorm(x, axis=-1, eps=1e-5):
    m = jnp.mean(x, axis=axis, keepdims=True)
    v = jnp.var(x, axis=axis, keepdims=True)
    return (x - m) / jnp.sqrt(v + eps)
def _scatter_add(tgt, idx, src, axis=0):
    return tgt.at[idx].add(src)
def _segment_sum(src, seg, n):
    return jax.ops.segment_sum(src, seg, n)
class _Rng:
    def __init__(self, key):
        self._k = key
    def _next(self):
        self._k, sub = jax.random.split(self._k)
        return sub
    def normal(self, shape):
        return jax.random.normal(self._next(), shape, dtype=jnp.bfloat16)
    def randint(self, lo, hi, shape):
        return jax.random.randint(self._next(), shape, lo, hi, dtype=jnp.int32)
    def uniform(self, shape, lo=0.0, hi=1.0):
        return jax.random.uniform(self._next(), shape, jnp.bfloat16, lo, hi)
    def permutation(self, n):
        return jax.random.permutation(self._next(), n)


kernel_name = 'standalone__modern_conv_block_slak__vision'

def setup_inputs():
    _rng = _Rng(jax.random.key(int.from_bytes(__import__("os").urandom(4), "little")))
    _w = (lambda a: (lambda t: t.astype(jnp.bfloat16) if jnp.issubdtype(t.dtype, jnp.floating) else t)(jnp.asarray(a)))
    H = W = 384
    C = 384
    K = 1
    return {
        "x": _w((lambda *s: _rng.normal(s) * 0.05)(1, H, W, C)),
        "dw": _w((lambda *s: _rng.normal(s) * 0.05)(K, K, C)),
        "w1": _w((lambda *s: _rng.normal(s) * 0.05)(C, 4 * C)),
        "w2": _w((lambda *s: _rng.normal(s) * 0.05)(4 * C, C)),
        "grn_g": _w((lambda *s: _rng.normal(s) * 0.05)(4 * C)),
        "grn_b": _w((lambda *s: _rng.normal(s) * 0.05)(4 * C)),
    }

def reference(x, dw, w1, w2, grn_g, grn_b):
    B, H, W, C = x.shape
    K = dw.shape[0]
    pad = K // 2
    xp = jnp.pad(x, ((0,0),(pad,pad),(pad,pad),(0,0)))
    out = jnp.zeros_like(x)
    for i in range(K):
        for j in range(K):
            out = out + xp[:, i:i+H, j:j+W, :] * dw[i, j][None, None, None, :]
    h = _layernorm(out, axis=-1)
    h = _gelu(h @ w1)
    gx = jnp.sqrt((h * h).sum(axis=(1, 2), keepdims=True) + 1e-6)
    nx = gx / (gx.mean(axis=-1, keepdims=True) + 1e-6)
    h = grn_g[None, None, None, :] * (h * nx) + grn_b[None, None, None, :] + h
    return x + h @ w2
```

```python
import functools
import math
import jax
import jax.numpy as jnp
from jax import lax
import jax.experimental.pallas as pl
import jax.experimental.pallas.tpu as pltpu

_A = math.sqrt(2.0 / math.pi)
_B = _A * 0.044715
_K = _B ** (1.0 / 3.0)
_C0 = _A / _K
_HS = 2.0 * _K


def build(TM=1024, NH=3, NX=3, NO=2, P=0, RM1=512, CN1=512, RM2=512, CK2=1536, LN_RM=None,
          vmem_mb=120, flags=None, only=0):
    LN_RM = LN_RM or RM1

    def kernel(x_hbm, dw_ref, w1_ref, w2_ref, g_ref, b_ref, o_hbm, h_hbm,
               xbuf, hbuf, obuf, xn_ref, w2s_ref, acc_ref, bias_ref, xsem, hsem, osem, *, nb, ns):
        C, D = w1_ref.shape

        def x_copy(i):
            s = i % NX
            return pltpu.make_async_copy(x_hbm.at[pl.ds(i * TM, TM)], xbuf.at[s], xsem.at[s])

        def o_copy(i):
            s = i % NO
            return pltpu.make_async_copy(obuf.at[s], o_hbm.at[pl.ds(i * TM, TM)], osem.at[s])

        def h_write(j):
            s = j % NH
            return pltpu.make_async_copy(hbuf.at[s], h_hbm.at[j], hsem.at[s])

        def h_read(j):
            s = j % NH
            return pltpu.make_async_copy(h_hbm.at[j], hbuf.at[s], hsem.at[s])

        def locate(i):
            if P == 0:
                return True, i, i % NH
            q, r = i // P, i % P
            streamed = r < P - 1
            j = q * (P - 1) + r
            return streamed, j, jnp.where(streamed, j % NH, NH + q)

        def when(c, f):
            if c is True:
                f()
            else:
                pl.when(c)(f)

        for i in range(NX):
            x_copy(i).start()
        acc_ref[...] = jnp.zeros_like(acc_ref)

        def phase1(i, carry):
            streamed, j, slot = locate(i)
            x_copy(i).wait()
            when(jnp.logical_and(streamed, j >= NH), lambda: h_write(j - NH).wait())
            xs = i % NX
            dw = dw_ref[...].astype(jnp.float32)
            for r in range(0, TM, LN_RM):
                y = xbuf[xs, pl.ds(r, LN_RM), :].astype(jnp.float32) * dw
                mu = jnp.sum(y, axis=-1, keepdims=True) * (1.0 / C)
                d = y - mu
                var = jnp.sum(d * d, axis=-1, keepdims=True) * (1.0 / C)
                xn_ref[pl.ds(r, LN_RM), :] = (d * (lax.rsqrt(var + 1e-5) * _K)).astype(jnp.bfloat16)
            for r in range(0, TM, RM1):
                a = xn_ref[pl.ds(r, RM1), :]
                for c in range(0, D, CN1):
                    z = jnp.dot(a, w1_ref[:, pl.ds(c, CN1)], preferred_element_type=jnp.float32)
                    t = jnp.tanh(z * (z * z + _C0))
                    h = z * t + z
                    acc_ref[:, pl.ds(c, CN1)] += jnp.sum((h * h).reshape(RM1 // 8, 8, CN1), axis=0)
                    hbuf[slot, pl.ds(r, RM1), pl.ds(c, CN1)] = h.astype(jnp.bfloat16)
            when(jnp.logical_and(streamed, j < ns - NH), lambda: h_write(j).start())
            when(i + NX < nb, lambda: x_copy(i + NX).start())
            return carry

        lax.fori_loop(0, nb, phase1, 0)

        ss = jnp.sum(acc_ref[...], axis=0, keepdims=True) * (1.0 / (_HS * _HS))
        gx = jnp.sqrt(ss + 1e-6)
        nx = gx / (jnp.sum(gx, axis=-1, keepdims=True) * (1.0 / D) + 1e-6)
        sc = (g_ref[...].astype(jnp.float32) * nx + 1.0) * (1.0 / _HS)
        sc_col = jnp.transpose(jnp.broadcast_to(sc, (128, D)))
        for c in range(0, C, 128):
            w2s_ref[:, pl.ds(c, 128)] = (w2_ref[:, pl.ds(c, 128)].astype(jnp.float32) * sc_col).astype(jnp.bfloat16)
        bias_ref[...] = jnp.dot(jnp.broadcast_to(b_ref[...], (16, D)), w2_ref[...],
                                preferred_element_type=jnp.float32)[:8]

        def phase2(k, carry):
            i = nb - 1 - k
            streamed, j, slot = locate(i)
            when(i < nb - NX, lambda: x_copy(i).wait())
            when(jnp.logical_and(streamed, j < ns - NH), lambda: h_read(j).wait())
            when(i + NO < nb, lambda: o_copy(i + NO).wait())
            xs, os_ = i % NX, i % NO
            bias = bias_ref[0:1, :]
            for r in range(0, TM, RM2):
                y = xbuf[xs, pl.ds(r, RM2), :].astype(jnp.float32) + bias
                for c in range(0, D, CK2):
                    y = y + jnp.dot(hbuf[slot, pl.ds(r, RM2), pl.ds(c, CK2)], w2s_ref[pl.ds(c, CK2), :],
                                    preferred_element_type=jnp.float32)
                obuf[os_, pl.ds(r, RM2), :] = y.astype(jnp.bfloat16)
            o_copy(i).start()
            when(jnp.logical_and(streamed, j >= NH), lambda: h_read(j - NH).start())
            when(i >= NX, lambda: x_copy(i - NX).start())
            return carry

        lax.fori_loop(0, nb, phase2, 0)
        for i in range(NO):
            o_copy(i).wait()

    @jax.jit
    def fn(x, dw, w1, w2, grn_g, grn_b):
        B, H, W, C = x.shape
        D = w1.shape[1]
        N = B * H * W
        nb = N // TM
        nr = nb // P if P else 0
        ns = nb - nr
        vm = pl.BlockSpec(memory_space=pltpu.VMEM)
        hbm = pl.BlockSpec(memory_space=pl.ANY)
        out, _ = pl.pallas_call(
            functools.partial(kernel, nb=nb, ns=ns),
            in_specs=[hbm, vm, vm, vm, vm, vm],
            out_specs=[hbm, hbm],
            out_shape=[jax.ShapeDtypeStruct((N, C), x.dtype),
                       jax.ShapeDtypeStruct((ns - NH, TM, D), jnp.bfloat16)],
            scratch_shapes=[
                pltpu.VMEM((NX, TM, C), x.dtype),
                pltpu.VMEM((NH + nr, TM, D), jnp.bfloat16),
                pltpu.VMEM((NO, TM, C), x.dtype),
                pltpu.VMEM((TM, C), jnp.bfloat16),
                pltpu.VMEM((D, C), jnp.bfloat16),
                pltpu.VMEM((8, D), jnp.float32),
                pltpu.VMEM((8, C), jnp.float32),
                pltpu.SemaphoreType.DMA((NX,)),
                pltpu.SemaphoreType.DMA((NH,)),
                pltpu.SemaphoreType.DMA((NO,)),
            ],
            compiler_params=pltpu.CompilerParams(vmem_limit_bytes=vmem_mb * 1024 * 1024, flags=flags),
            name="slak_block",
        )(x.reshape(N, C), dw.reshape(1, C), w1, w2, grn_g.reshape(1, D), grn_b.reshape(1, D))
        return out.reshape(B, H, W, C)

    return fn


_fn = build(TM=1024,P=5,RM1=256,RM2=256)


def pallas_standalone__modern_conv_block_slak__vision_kernel(x, dw, w1, w2, grn_g, grn_b):
    return _fn(x, dw, w1, w2, grn_g, grn_b)


pallas_standalone__modern_conv_block_slak__vision_kernel = jax.jit(
    pallas_standalone__modern_conv_block_slak__vision_kernel)
```

```python
import functools
import math
import jax
import jax.numpy as jnp
from jax import lax
import jax.experimental.pallas as pl
import jax.experimental.pallas.tpu as pltpu

_A = math.sqrt(2.0 / math.pi)
_B = _A * 0.044715
_K = _B ** (1.0 / 3.0)
_C0 = _A / _K
_HS = 2.0 * _K
F32, BF16, U32 = jnp.float32, jnp.bfloat16, jnp.uint32


def build(TM=3584, TS=3072, TF=512, NH=2, NX=2, NO=2, RM1=128, CN1=512, RM2=256, CK2=1536, LNR=None, LA=None,
          DP=1024, DP1=None, XR=4, vmem_mb=120, flags=None, nobc=False, lnpos=0, tail1=None, tail2=None, its=False):
    LNR = LNR or RM1
    LA = LA or RM1
    DP1 = DP1 or DP
    TR = TM - TS

    def chunks(rm, bounds, tail=None):
        out = []
        for lo, hi in bounds:
            r = lo
            while r < hi:
                m = min(rm, hi - r)
                out.append((r, m))
                r += m
        if tail:
            r, m = out.pop()
            assert sum(tail) == m
            for t in tail:
                out.append((r, t))
                r += t
        return out

    pieces = lambda n, dp: [(r, min(dp, n - r)) for r in range(0, n, dp)]

    def kernel(x_hbm, dw_ref, w1_hbm, w2_hbm, g_ref, b_ref, o_hbm, h_hbm,
               xbuf, xf, hbuf, hres, hf, obuf, xn_ref, xn0_ref, w1_raw, w2_raw, w1_ref, w2_ref, acc_ref, bias_ref,
               xsem, x0sem, hsem, osem, wsem, *, nb):
        C, D = w1_hbm.shape

        def rows(i, r, m):
            return pl.ds(pl.multiple_of(TF + i * TM + r, 16), m)

        x_copy = lambda i, s, r, m, sem: pltpu.make_async_copy(
            x_hbm.at[rows(i, r, m)], xbuf.at[s, pl.ds(r, m)], sem.at[s])
        x_head = lambda i, s: x_copy(i, s, 0, LA, x0sem)
        x_rest = lambda i, s: x_copy(i, s, LA, TM - LA, xsem)
        x_full = lambda i, s: x_copy(i, s, 0, TM, xsem)
        o_copy = lambda i, s, r=0, m=TM: pltpu.make_async_copy(
            obuf.at[s, pl.ds(r, m)], o_hbm.at[rows(i, r, m)], osem.at[s])
        h_write = lambda i, s, r=0, m=TS: pltpu.make_async_copy(
            hbuf.at[s, pl.ds(r // 2, m // 2)], h_hbm.at[i, pl.ds(r // 2, m // 2)], hsem.at[s])
        h_read = lambda i, s, r=0, m=TS: pltpu.make_async_copy(
            h_hbm.at[i, pl.ds(r // 2, m // 2)], hbuf.at[s, pl.ds(r // 2, m // 2)], hsem.at[s])
        w1_copy = pltpu.make_async_copy(w1_hbm, w1_raw, wsem.at[0])
        w2_copy = pltpu.make_async_copy(w2_hbm, w2_raw, wsem.at[1])
        xf_in = pltpu.make_async_copy(x_hbm.at[pl.ds(0, TF)], xf, wsem.at[2])
        xf_out = pltpu.make_async_copy(xf, o_hbm.at[pl.ds(0, TF)], wsem.at[2])

        def layernorm(src, r, m):
            y = src[pl.ds(r, m), :].astype(F32) * dw_ref[...].astype(F32)
            mu = jnp.sum(y, axis=-1, keepdims=True) * (1.0 / C)
            d = y - mu
            var = jnp.sum(d * d, axis=-1, keepdims=True) * (1.0 / C)
            return (d * (lax.rsqrt(var + 1e-5) * _K)).astype(BF16)

        def expand(a, out_fn, after=None):
            m = a.shape[0]
            for c in range(0, D, CN1):
                z = jnp.dot(a, pltpu.bitcast(w1_ref[:, pl.ds(c, CN1)], BF16), preferred_element_type=F32)
                t = jnp.tanh(z * (z * z + _C0))
                h = z * t + z
                acc_ref[:, pl.ds(c, CN1)] += jnp.sum((h * h).reshape(m // 8, 8, CN1), axis=0)
                out_fn(c, pltpu.bitcast(h.astype(BF16), U32))

        def project(xv, hv):
            m = xv.shape[0]
            y = (xv.astype(F32).reshape(m // 8, 8, C) + bias_ref[...]).reshape(m, C)
            for c in range(0, D, CK2):
                y = y + jnp.dot(pltpu.bitcast(hv[:, pl.ds(c, CK2)], BF16),
                                pltpu.bitcast(w2_ref[pl.ds(c // 2, CK2 // 2), :], BF16), preferred_element_type=F32)
            return y.astype(BF16)

        def h_view(i, s, r, m):
            if r < TS:
                return hbuf.at[s, pl.ds(r // 2, m // 2)]
            return hres.at[i, pl.ds((r - TS) // 2, m // 2)]

        def store_cols(ref):
            def put(c, v):
                ref[:, pl.ds(c, CN1)] = v
            return put

        nxt = lambda s, n: jnp.where(s == n - 1, 0, s + 1)
        prv = lambda s, n: jnp.where(s == 0, n - 1, s - 1)

        with jax.named_scope('pro'):
            w1_copy.start()
            xf_in.start()
            x_head(0, 0).start()
            acc_ref[...] = jnp.zeros_like(acc_ref)
            xf_in.wait()
            x_head(0, 0).wait()
            w1_copy.wait()
            x_rest(0, 0).start()
            for i in range(1, NX):
                x_head(i, i).start()
            w1_ref[...] = pltpu.bitcast(w1_raw[...], U32)
            for r, m in chunks(RM1, [(0, TF)]):
                expand(layernorm(xf, r, m), store_cols(hf.at[pl.ds(r // 2, m // 2)]))
            for r in range(0, LA, LNR):
                xn0_ref[pl.ds(r, LNR), :] = layernorm(xbuf.at[0], r, LNR)
            for i in range(1, NX):
                x_rest(i, i).start()
            w2_copy.start()

        RING = XR * RM1

        def phase1(i, carry):
            xs, hs = carry
            xn_s = nxt(xs, NX)
            x_rest(i, xs).wait()
            pl.when(i + 1 < nb)(lambda: x_head(i + 1, xn_s).wait())
            pl.when(i >= NH)(lambda: h_write(i - NH, hs).wait())
            pl.when(i + NX < nb)(lambda: x_head(i + NX, xs).start())
            ln_rows = list(range(LA, TM + LA, LNR))
            hp = pieces(TS, DP1)

            def ln_upto(lim):
                while ln_rows and ln_rows[0] < lim:
                    q = ln_rows.pop(0)
                    if q < TM:
                        xn_ref[pl.ds(q % RING, LNR), :] = layernorm(xbuf.at[xs], q, LNR)
                    else:
                        xn0_ref[pl.ds(q - TM, LNR), :] = layernorm(xbuf.at[xn_s], q - TM, LNR)

            for r, m in chunks(RM1, [(0, TS), (TS, TM)], tail1):
                a = xn0_ref[pl.ds(r, m), :] if r < LA else xn_ref[pl.ds(r % RING, m), :]
                if lnpos == 0:
                    ln_upto(r + m + LA)
                expand(a, store_cols(h_view(i, hs, r, m)))
                if lnpos == 1:
                    ln_upto(r + m + LA)
                while hp and hp[0][0] + hp[0][1] <= r + m:
                    pr, pm = hp.pop(0)
                    pl.when(i < nb - NH)(lambda: h_write(i, hs, pr, pm).start())
            pl.when(i + NX < nb)(lambda: x_rest(i + NX, xs).start())
            return xn_s, nxt(hs, NH)

        def scoped(f, name):
            if not its:
                return f
            def g(i, c):
                with jax.named_scope(name):
                    return f(i, c)
            return g

        with jax.named_scope('ph1'):
            lax.fori_loop(0, nb, scoped(phase1, 'it1'), (jnp.int32(0), jnp.int32(0)))

        with jax.named_scope('mid'):
            w2_copy.wait()
            nt = D // 128
            row = lambda ref: jnp.concatenate([ref[k:k + 1, :] for k in range(nt)], axis=1)
            g = row(g_ref[...].astype(F32))
            b = row(b_ref[...].astype(F32))
            bias_ref[...] = jnp.dot(jnp.broadcast_to(b, (16, D)).astype(BF16), w2_raw[...],
                                    preferred_element_type=F32)[:8]
            ss = jnp.sum(acc_ref[...], axis=0, keepdims=True) * (1.0 / (_HS * _HS))
            gx = jnp.sqrt(ss + 1e-6)
            nx = gx / (jnp.sum(gx, axis=-1, keepdims=True) * (1.0 / D) + 1e-6)
            sc = (g * nx + 1.0) * (1.0 / _HS)
            for k in range(nt):
                col = jnp.transpose(jnp.broadcast_to(sc[:, k * 128:(k + 1) * 128], (128, 128)))
                for c in range(0, C, 128):
                    v = (w2_raw[pl.ds(k * 128, 128), pl.ds(c, 128)].astype(F32) * col).astype(BF16)
                    w2_ref[pl.ds(k * 64, 64), pl.ds(c, 128)] = pltpu.bitcast(v, U32)

        def phase2(k, carry):
            xs, hs, os_ = carry
            i = nb - 1 - k
            pl.when(k >= NX)(lambda: x_full(i, xs).wait())
            pl.when(k >= NH)(lambda: h_read(i, hs).wait())
            pl.when(k >= NO)(lambda: o_copy(i + NO, os_).wait())
            hp, op = pieces(TS, DP), pieces(TM, DP)
            for r, m in chunks(RM2, [(0, TS), (TS, TM)], tail2):
                obuf[os_, pl.ds(r, m), :] = project(xbuf[xs, pl.ds(r, m), :], h_view(i, hs, r, m))
                while hp and hp[0][0] + hp[0][1] <= r + m:
                    pr, pm = hp.pop(0)
                    pl.when(i >= NH)(lambda: h_read(i - NH, hs, pr, pm).start())
                while op and op[0][0] + op[0][1] <= r + m:
                    pr, pm = op.pop(0)
                    o_copy(i, os_, pr, pm).start()
                    pl.when(i >= NX)(lambda: x_copy(i - NX, xs, pr, pm, xsem).start())
            return prv(xs, NX), prv(hs, NH), prv(os_, NO)

        with jax.named_scope('ph2'):
            lax.fori_loop(0, nb, scoped(phase2, 'it2'), tuple(jnp.int32((nb - 1) % n) for n in (NX, NH, NO)))
        with jax.named_scope('epi'):
            for r, m in chunks(RM2, [(0, TF)]):
                xf[pl.ds(r, m), :] = project(xf[pl.ds(r, m), :], hf.at[pl.ds(r // 2, m // 2)])
            xf_out.start()
            for i in range(NO):
                o_copy(i, i).wait()
            xf_out.wait()

    @jax.jit
    def fn(x, dw, w1, w2, grn_g, grn_b):
        B, H, W, C = x.shape
        D = w1.shape[1]
        N = B * H * W
        nb = (N - TF) // TM
        assert nb * TM + TF == N
        vm = pl.BlockSpec(memory_space=pltpu.VMEM)
        hbm = pl.BlockSpec(memory_space=pl.ANY)
        out, _ = pl.pallas_call(
            functools.partial(kernel, nb=nb),
            in_specs=[hbm, vm, hbm, hbm, vm, vm],
            out_specs=[hbm, hbm],
            out_shape=[jax.ShapeDtypeStruct((N, C), x.dtype),
                       jax.ShapeDtypeStruct((nb - NH, TS // 2, D), U32)],
            scratch_shapes=[
                pltpu.VMEM((NX, TM, C), x.dtype),
                pltpu.VMEM((TF, C), x.dtype),
                pltpu.VMEM((NH, TS // 2, D), U32),
                pltpu.VMEM((nb, TR // 2, D) if TR else (1, 8, 128), U32),
                pltpu.VMEM((TF // 2, D), U32),
                pltpu.VMEM((NO, TM, C), x.dtype),
                pltpu.VMEM((XR * RM1, C), BF16),
                pltpu.VMEM((LA, C), BF16),
                pltpu.VMEM((C, D), BF16),
                pltpu.VMEM((D, C), BF16),
                pltpu.VMEM((C // 2, D), U32),
                pltpu.VMEM((D // 2, C), U32),
                pltpu.VMEM((8, D), F32),
                pltpu.VMEM((8, C), F32),
                pltpu.SemaphoreType.DMA((NX,)),
                pltpu.SemaphoreType.DMA((NX,)),
                pltpu.SemaphoreType.DMA((NH,)),
                pltpu.SemaphoreType.DMA((NO,)),
                pltpu.SemaphoreType.DMA((3,)),
            ],
            compiler_params=pltpu.CompilerParams(vmem_limit_bytes=vmem_mb * 1024 * 1024, flags=flags,
                                                 disable_bounds_checks=nobc),
            name="slak_block",
        )(x.reshape(N, C), dw.reshape(1, C), w1, w2, grn_g.reshape(D // 128, 128), grn_b.reshape(D // 128, 128))
        return out.reshape(B, H, W, C)

    return fn


_fn = build(TM=3200,TS=2816,TF=256,tail1=(64,64))


def pallas_standalone__modern_conv_block_slak__vision_kernel(x, dw, w1, w2, grn_g, grn_b):
    return _fn(x, dw, w1, w2, grn_g, grn_b)


pallas_standalone__modern_conv_block_slak__vision_kernel = jax.jit(
    pallas_standalone__modern_conv_block_slak__vision_kernel)
```

```python
import functools
import math
import numpy as np
import jax
import jax.numpy as jnp
from jax import lax
import jax.experimental.pallas as pl
import jax.experimental.pallas.tpu as pltpu

_A = math.sqrt(2.0 / math.pi)
_B = _A * 0.044715
_K = _B ** (1.0 / 3.0)
_C0 = _A / _K
_HS = 2.0 * _K
F32, BF16, U32 = jnp.float32, jnp.bfloat16, jnp.uint32

_RHS = (
    ((+1, 1, 0), (-1, 2, 0), (+1, 2, 2)),
    ((+1, 1, 0),),
    ((+1, 0, 0), (+1, 2, 0), (+1, 2, 1)),
    ((+1, 0, 1),),
    ((+1, 1, 0), (+1, 2, 1)),
    ((+1, 0, 0),),
    ((+1, 2, 1),),
    ((+1, 1, 1), (-1, 1, 2), (-1, 2, 1)),
    ((+1, 1, 2),),
    ((+1, 0, 1), (+1, 1, 0), (+1, 1, 1)),
    ((+1, 2, 2),),
    ((+1, 0, 0), (+1, 2, 2)),
    ((+1, 0, 1), (+1, 1, 2)),
    ((-1, 0, 1), (+1, 0, 2), (+1, 2, 2)),
    ((-1, 0, 0), (+1, 0, 2), (+1, 1, 2)),
)


def _lhs(a):
    memo = {}

    def get(r):
        if r not in memo:
            memo[r] = {
                1: lambda: a(1, 1) + a(1, 2),
                3: lambda: a(0, 0) - a(0, 1),
                4: lambda: get(1) - a(0, 1),
                5: lambda: a(0, 0) - a(0, 2),
                6: lambda: get(4) - a(0, 2),
                7: lambda: a(1, 1) - a(0, 1),
                8: lambda: a(1, 0) - a(1, 1),
                10: lambda: get(11) + a(1, 2),
                11: lambda: get(5) - a(1, 0),
                12: lambda: a(1, 0) - a(0, 1),
                13: lambda: a(0, 0) - a(1, 0),
            }[r]()
        return memo[r]
    return get


_PLAIN = {0: (1, 2), 2: (0, 2), 9: (0, 1), 14: (1, 0)}
_ORDER = (1, 4, 9, 6, 5, 2, 3, 11, 0, 10, 14, 8, 12, 13, 7)
_LAST = (1, 1)


def _combine(prod, emit):
    m1 = prod(1)
    p = m1 - prod(4)
    q = prod(9) - p
    m6 = prod(6)
    m5 = prod(5)
    emit(0, 0, prod(2) + ((m5 + m6) + p))
    m3 = prod(3)
    emit(0, 1, m3 + (q - m6))
    s = prod(11) - m5
    m0 = prod(0)
    m10 = prod(10)
    emit(1, 0, m10 + ((m1 - m0) - s))
    t = prod(14) - s
    m8 = prod(8)
    emit(1, 2, (m10 + t) - m8)
    m12 = prod(12)
    emit(0, 2, prod(13) + ((m3 - m12) + t))
    emit(1, 1, prod(7) + ((m12 - m8) + q))


def _plan(nb, S, NH, LO, U, LX, rho, beta):
    keep, order = list(range(NH, S)), []
    stream = list(range(S, nb))
    n = nb - NH
    for t in range(n):
        due = (t + 1) * (S - NH) // n > t * (S - NH) // n
        order.append(keep.pop() if due else stream.pop())
    order += list(range(NH - 1, -1, -1))
    when = {k: t // U for t, k in enumerate(order)}
    busy = {s: [(when[s] - LX, when[s])] for s in range(NH)}
    rows, dirty, c = [], set(), 0
    for t, k in enumerate(order):
        if k < S:
            xs = hs = k
        else:
            lo, hi = t // U - LX, t // U
            xs = next(s for s in busy if all(b < lo or a > hi for a, b in busy[s]))
            busy[xs].append((lo, hi))
            hs, c = c % NH, c + 1
        rows.append((k, xs, hs, int(hs in dirty), int(k >= S)))
        if k >= S:
            dirty.add(hs)
    rows += [rows[-1]] * (U * LX)
    fetch, j = [], S
    for k in range(len(rows)):
        go = j < nb and j - S <= k and (j - S < rho * k + beta or j - k <= 3)
        fetch.append(j if go else 0)
        j += go
    assert j == nb and all(f == 0 or f - k >= 2 for k, f in enumerate(fetch))
    return np.asarray([r + (f,) for r, f in zip(rows, fetch)], np.int32).T.copy()


def build(TB=1024, U=2, S=31, NH=6, LO=2, LX=2, R1=128, R2=128, LNR=16, lnhook=(0, 32), lead=2, DP=512, rho=0.8, beta=5,
          vmem_mb=127, flags=None, nobc=True, its=False):
    M1, M2 = 2 * R1, 2 * R2
    SX = S + LO
    assert TB % M1 == 0 and TB % M2 == 0 and (U * TB // M1) % 2 == 0

    def kernel(tab, x_hbm, dw_ref, w1_hbm, w2_hbm, g_ref, b_ref, o_hbm, h_hbm,
               xbuf, hbuf, ring0, ring1, wc, acc_ref, bias_ref, pin_ref, xsem, x0sem, hsem, osem, wsem, *, nb):
        C, D = w1_hbm.shape
        G = D // 3
        ring = (ring0, ring1)

        rows = lambda k, r, m: pl.ds(pl.multiple_of(k * TB + r, 16), m)
        x_copy = lambda k, s, r, m, sem: pltpu.make_async_copy(
            x_hbm.at[rows(k, r, m)], xbuf.at[rows(s, r, m)], sem.at[s])
        x_head = lambda k, s: x_copy(k, s, 0, M1, x0sem)
        x_rest = lambda k, s: x_copy(k, s, M1, TB - M1, xsem)
        x_full = lambda k, s: x_copy(k, s, 0, TB, xsem)
        o_copy = lambda k, s, r=0, m=TB: pltpu.make_async_copy(
            xbuf.at[rows(s, r, m)], o_hbm.at[rows(k, r, m)], osem.at[s])
        h_write = lambda k, s: pltpu.make_async_copy(hbuf.at[s], h_hbm.at[k - S], hsem.at[s])
        h_read = lambda k, s, r=0, m=TB: pltpu.make_async_copy(
            h_hbm.at[k - S, pl.ds(r // 2, m // 2)], hbuf.at[s, pl.ds(r // 2, m // 2)], hsem.at[s])
        W0 = S * TB
        w1_copy = [pltpu.make_async_copy(w1_hbm.at[:, pl.ds(q * C, C)], xbuf.at[pl.ds(W0 + q * C, C)], wsem.at[q])
                   for q in range(D // C)]
        w1_tile = lambda r, c: xbuf[pl.ds(W0 + c // C * C + r, 128), pl.ds(c % C, 128)]
        w2_ref = xbuf.at[pl.ds(W0, D)]
        w2_copy = pltpu.make_async_copy(w2_hbm, w2_ref, wsem.at[0])

        def layernorm(xv):
            y = xv * dw_ref[...].astype(F32)
            mu = jnp.sum(y, axis=-1, keepdims=True) * (1.0 / C)
            d = y - mu
            var = jnp.sum(d * d, axis=-1, keepdims=True)
            return d * (lax.rsqrt(var + 1e-5 * C) * (_K * math.sqrt(C)))

        def normalise(s, r, q, dst):
            words = [pltpu.bitcast(xbuf[rows(s, r + i * R1 + q, LNR), :], U32) for i in range(2)]
            combos = []
            for parity in range(2):
                halves = [layernorm(pltpu.unpack_elementwise(w, index=parity, packed_dtype=BF16, unpacked_dtype=F32))
                          for w in words]
                blk = lambda i, k, halves=halves: halves[i][:, k * 128:(k + 1) * 128]
                lhs = _lhs(blk)
                combos.append({p: blk(*_PLAIN[p]) if p in _PLAIN else lhs(p) for p in _ORDER})
            for p in _ORDER:
                v = pltpu.pack_elementwise([combos[0][p], combos[1][p]], packed_dtype=BF16)
                dst[pl.ds((p * R1 + q) // 2, LNR // 2), :] = pltpu.bitcast(v, U32)

        def expand(src, hv, todo):
            for c in range(0, G, 128):
                def prod(p):
                    return jnp.dot(pltpu.bitcast(src[pl.ds(p * R1 // 2, R1 // 2), :], BF16),
                                   pltpu.bitcast(wc[p, pl.ds(c // 2, 64), :], BF16), preferred_element_type=F32)

                def emit(i, j, z):
                    t = jnp.tanh(z * (z * z + _C0))
                    h = z * t + z
                    cols = pl.ds(j * G + c, 128)
                    acc_ref[:, cols] += jnp.sum((h * h).reshape(R1 // 8, 8, 128), axis=0)
                    hv[pl.ds(i * R1 // 2, R1 // 2), cols] = pltpu.bitcast(h.astype(BF16), U32)
                    if (i, j) == _LAST:
                        for g in lnhook:
                            if todo:
                                xbuf[pl.ds(SX * TB, 8), pl.ds(0, 128)] = z[g:g + 8].astype(BF16)
                                todo.pop(0)()

                _combine(prod, emit)

        def project(s, hv, r):
            raw = lambda i, k: pltpu.bitcast(hv[pl.ds((r + i * R2) // 2, R2 // 2), pl.ds(k * G, G)], BF16)
            lhs = _lhs(lambda i, k: raw(i, k).astype(F32))
            xv = xbuf.at[rows(s, r, M2)]

            def prod(p):
                a = raw(*_PLAIN[p]) if p in _PLAIN else lhs(p).astype(BF16)
                return jnp.dot(a, pltpu.bitcast(wc[p], BF16), preferred_element_type=F32)

            def emit(i, j, y):
                blk = (pl.ds(i * R2, R2), pl.ds(j * 128, 128))
                res = xv[blk].astype(F32).reshape(R2 // 8, 8, 128) + bias_ref[:, pl.ds(j * 128, 128)]
                xv[blk] = (res.reshape(R2, 128) + y).astype(BF16)

            _combine(prod, emit)

        def rhs(blk):
            for q in range(0, G, 128):
                b = {(k, j): blk(k, j, q) for k in range(3) for j in range(3)}
                for p, terms in enumerate(_RHS):
                    v = None
                    for sign, k, j in sorted(terms, reverse=True):
                        v = b[k, j] if v is None else (v + b[k, j] if sign > 0 else v - b[k, j])
                    wc[p, pl.ds(q // 2, 64), :] = pltpu.bitcast(v.astype(BF16), U32)

        def scoped(f, name):
            if not its:
                return f

            def g(i, c):
                with jax.named_scope(name):
                    return f(i, c)
            return g

        def fetch(t):
            x_head(tab[0, t], tab[1, t]).start()
            x_rest(tab[0, t], tab[1, t]).start()

        with jax.named_scope('pro'):
            for cp in w1_copy:
                cp.start()
            fetch(0)
            acc_ref[...] = jnp.zeros_like(acc_ref)
            for t in range(1, U * LX):
                fetch(t)
            for cp in w1_copy:
                cp.wait()
            rhs(lambda k, j, q: w1_tile(k * 128, j * G + q).astype(F32))
            w2_copy.start()
            x_head(tab[0, 0], tab[1, 0]).wait()
            for q in range(0, R1, LNR):
                normalise(tab[1, 0], 0, q, ring[0])

        def phase1(it, carry):
            t0 = it * U
            blk = [tab[0, t0 + u] for u in range(U + 1)]
            xs = [tab[1, t0 + u] for u in range(U + 1)]
            hs = [tab[2, t0 + u] for u in range(U)]
            for u in range(U):
                x_rest(blk[u], xs[u]).wait()
                if u + 1 < U:
                    x_head(blk[u + 1], xs[u + 1]).wait()
                else:
                    pl.when(t0 + U < nb)(lambda: x_head(blk[U], xs[U]).wait())
                pl.when(tab[3, t0 + u] > 0)(lambda: h_write(S, hs[u]).wait())
            for u in range(U):
                pl.when(t0 + U * LX + u < nb)(functools.partial(fetch, t0 + U * LX + u))
            zero = pl.multiple_of((it >> 20) * 8, 8)

            def piece(n):
                c, q = divmod(n, R1 // LNR)
                u, r = divmod((c + 1) * M1, TB)
                dst = ring[(c + 1) % 2]
                normalise(xs[u], r, q * LNR, dst)
                pin_ref[n] = dst[pl.ds(zero, 8), :]

            todo = [functools.partial(piece, n) for n in range(U * TB // (2 * LNR))]
            for _ in range(lead):
                todo.pop(0)()
            for c in range(U * TB // M1):
                u, r = divmod(c * M1, TB)
                expand(ring[c % 2], hbuf.at[hs[u], pl.ds(r // 2, R1)], todo)
                assert len(todo) <= (U * TB - (c + 1) * M1) // (2 * LNR)
                if r + M1 == TB:
                    pl.when(tab[4, t0 + u] > 0)(lambda: h_write(blk[u], hs[u]).start())
            return carry

        with jax.named_scope('ph1'):
            lax.fori_loop(0, nb // U, scoped(phase1, 'it1'), 0)

        with jax.named_scope('mid'):
            w2_copy.wait()
            nt = D // 128
            row = lambda ref: jnp.concatenate([ref[k:k + 1, :] for k in range(nt)], axis=1)
            g = row(g_ref[...].astype(F32))
            b = jnp.broadcast_to(row(b_ref[...].astype(F32)), (16, D)).astype(BF16)
            bias_ref[...] = jnp.dot(b, w2_ref[...], preferred_element_type=F32)[:8]
            ss = jnp.sum(acc_ref[...], axis=0, keepdims=True) * (1.0 / (_HS * _HS))
            gx = jnp.sqrt(ss + 1e-6)
            nx = gx / (jnp.sum(gx, axis=-1, keepdims=True) * (1.0 / D) + 1e-6)
            sc = (g * nx + 1.0) * (1.0 / _HS)
            col = functools.lru_cache(None)(
                lambda r: jnp.transpose(jnp.broadcast_to(sc[:, r:r + 128], (128, 128))))
            rhs(lambda k, j, q: w2_ref[pl.ds(k * G + q, 128), pl.ds(j * 128, 128)].astype(F32) * col(k * G + q))
            for k in range(S, SX):
                x_full(k, k).start()

        nxt = lambda s, n: jnp.where(s == n - 1, 0, s + 1)

        def phase2(k, carry):
            xs, hs, ps = carry

            @pl.when(k >= S)
            def _():
                h_read(k, hs).wait()
                x_full(k, xs).wait()
            pl.when(k >= LO)(lambda: o_copy(k - LO, ps).wait())
            j = tab[5, k]
            jx, jh = lax.rem(j, SX), lax.rem(j, S)
            pl.when(j >= SX)(lambda: x_full(j, jx).start())
            done = 0
            for r in range(0, TB, M2):
                project(xs, hbuf.at[hs], r)
                if r + M2 - done >= DP or r + M2 == TB:
                    pl.when(j > 0)(lambda: h_read(j, jh, done, r + M2 - done).start())
                    o_copy(k, xs, done, r + M2 - done).start()
                    done = r + M2
            return nxt(xs, SX), nxt(hs, S), nxt(ps, SX)

        with jax.named_scope('ph2'):
            lax.fori_loop(0, nb, scoped(phase2, 'it2'), (jnp.int32(0), jnp.int32(0), jnp.int32(S)))
        with jax.named_scope('epi'):
            for k in range(nb - LO, nb):
                o_copy(k, k % SX).wait()

    @jax.jit
    def fn(x, dw, w1, w2, grn_g, grn_b):
        B, H, W, C = x.shape
        D = w1.shape[1]
        N = B * H * W
        nb = N // TB
        assert nb * TB == N and nb % U == 0 and LO * TB >= D
        tab = _plan(nb, S, NH, LO, U, LX, rho, beta)
        vm = pl.BlockSpec(memory_space=pltpu.VMEM)
        hbm = pl.BlockSpec(memory_space=pl.ANY)
        out, _ = pl.pallas_call(
            functools.partial(kernel, nb=nb),
            in_specs=[pl.BlockSpec(memory_space=pltpu.SMEM), hbm, vm, hbm, hbm, vm, vm],
            out_specs=[hbm, hbm],
            out_shape=[jax.ShapeDtypeStruct((N, C), x.dtype),
                       jax.ShapeDtypeStruct((nb - S, TB // 2, D), U32)],
            scratch_shapes=[
                pltpu.VMEM((SX * TB + 64, C), x.dtype),
                pltpu.VMEM((S, TB // 2, D), U32),
                pltpu.VMEM((15 * R1 // 2, 128), U32),
                pltpu.VMEM((15 * R1 // 2, 128), U32),
                pltpu.VMEM((15, D // 6, 128), U32),
                pltpu.VMEM((8, D), F32),
                pltpu.VMEM((8, C), F32),
                pltpu.VMEM((U * TB // (2 * LNR), 8, 128), U32),
                pltpu.SemaphoreType.DMA((SX,)),
                pltpu.SemaphoreType.DMA((SX,)),
                pltpu.SemaphoreType.DMA((S,)),
                pltpu.SemaphoreType.DMA((SX,)),
                pltpu.SemaphoreType.DMA((D // C,)),
            ],
            compiler_params=pltpu.CompilerParams(vmem_limit_bytes=int(vmem_mb * 1024 * 1024), flags=flags,
                                                 disable_bounds_checks=nobc),
            name="slak_block",
        )(tab, x.reshape(N, C), dw.reshape(1, C), w1, w2,
          grn_g.reshape(D // 128, 128), grn_b.reshape(D // 128, 128))
        return out.reshape(B, H, W, C)

    return fn


_fn = build(S=32,NH=12,U=3,vmem_mb=127.9,DP=1024)


def pallas_standalone__modern_conv_block_slak__vision_kernel(x, dw, w1, w2, grn_g, grn_b):
    return _fn(x, dw, w1, w2, grn_g, grn_b)


pallas_standalone__modern_conv_block_slak__vision_kernel = jax.jit(
    pallas_standalone__modern_conv_block_slak__vision_kernel)
```

```python
import functools
import math
import numpy as np
import jax
import jax.numpy as jnp
from jax import lax
import jax.experimental.pallas as pl
import jax.experimental.pallas.tpu as pltpu

_A = math.sqrt(2.0 / math.pi)
_B = _A * 0.044715
_K = _B ** (1.0 / 3.0)
_C0 = _A / _K
_HS = 2.0 * _K
F32, BF16, U32 = jnp.float32, jnp.bfloat16, jnp.uint32

_RHS = (
    ((+1, 1, 0), (-1, 2, 0), (+1, 2, 2)),
    ((+1, 1, 0),),
    ((+1, 0, 0), (+1, 2, 0), (+1, 2, 1)),
    ((+1, 0, 1),),
    ((+1, 1, 0), (+1, 2, 1)),
    ((+1, 0, 0),),
    ((+1, 2, 1),),
    ((+1, 1, 1), (-1, 1, 2), (-1, 2, 1)),
    ((+1, 1, 2),),
    ((+1, 0, 1), (+1, 1, 0), (+1, 1, 1)),
    ((+1, 2, 2),),
    ((+1, 0, 0), (+1, 2, 2)),
    ((+1, 0, 1), (+1, 1, 2)),
    ((-1, 0, 1), (+1, 0, 2), (+1, 2, 2)),
    ((-1, 0, 0), (+1, 0, 2), (+1, 1, 2)),
)


def _lhs(a):
    memo = {}

    def get(r):
        if r not in memo:
            memo[r] = {
                1: lambda: a(1, 1) + a(1, 2),
                3: lambda: a(0, 0) - a(0, 1),
                4: lambda: get(1) - a(0, 1),
                5: lambda: a(0, 0) - a(0, 2),
                6: lambda: get(4) - a(0, 2),
                7: lambda: a(1, 1) - a(0, 1),
                8: lambda: a(1, 0) - a(1, 1),
                10: lambda: get(11) + a(1, 2),
                11: lambda: get(5) - a(1, 0),
                12: lambda: a(1, 0) - a(0, 1),
                13: lambda: a(0, 0) - a(1, 0),
            }[r]()
        return memo[r]
    return get


_PLAIN = {0: (1, 2), 2: (0, 2), 9: (0, 1), 14: (1, 0)}
_ORDER = (1, 4, 9, 6, 5, 2, 3, 11, 0, 10, 14, 8, 12, 13, 7)
_SHARED = {"p": (1, 4), "q": (9, "p"), "s": (11, 5), "t": (14, "s")}
_OUTS = {
    (0, 0): ((+1, 2), (+1, 5), (+1, 6), (+1, "p")),
    (0, 1): ((+1, 3), (+1, "q"), (-1, 6)),
    (1, 0): ((+1, 10), (+1, 1), (-1, 0), (-1, "s")),
    (1, 2): ((+1, 10), (+1, "t"), (-1, 8)),
    (0, 2): ((+1, 13), (+1, 3), (-1, 12), (+1, "t")),
    (1, 1): ((+1, 7), (+1, 12), (-1, 8), (+1, "q")),
}


def _combine(prod, emit, order=_ORDER):
    have, left = {}, dict(_OUTS)
    for r in order:
        have[r] = prod(r)
        for name, (u, v) in _SHARED.items():
            if name not in have and u in have and v in have:
                have[name] = have[u] - have[v]
        for out, terms in list(left.items()):
            if all(key in have for _, key in terms):
                age = list(have)
                terms = sorted(terms, key=lambda term: age.index(term[1]))
                sign, val = terms[0][0], have[terms[0][1]]
                for s, key in terms[1:]:
                    if s == sign:
                        val = val + have[key]
                    else:
                        sign, val = +1, (val - have[key] if sign > 0 else have[key] - val)
                assert sign > 0
                emit(*out, val)
                del left[out]


def _plan(nb, S, NH, LO, U, LX, rho, beta):
    keep, order = list(range(NH, S)), []
    stream = list(range(S, nb))
    n = nb - NH
    for t in range(n):
        due = (t + 1) * (S - NH) // n > t * (S - NH) // n
        order.append(keep.pop() if due else stream.pop())
    order += list(range(NH - 1, -1, -1))
    when = {k: t // U for t, k in enumerate(order)}
    busy = {s: [(when[s] - LX, when[s])] for s in range(NH)}
    rows, dirty, c = [], set(), 0
    for t, k in enumerate(order):
        if k < S:
            xs = hs = k
        else:
            lo, hi = t // U - LX, t // U
            xs = next(s for s in busy if all(b < lo or a > hi for a, b in busy[s]))
            busy[xs].append((lo, hi))
            hs, c = c % NH, c + 1
        rows.append((k, xs, hs, int(hs in dirty), int(k >= S)))
        if k >= S:
            dirty.add(hs)
    rows += [rows[-1]] * (U * LX)
    fetch, j = [], S
    for k in range(len(rows)):
        go = j < nb and j - S <= k and (j - S < rho * k + beta or j - k <= 3)
        fetch.append(j if go else 0)
        j += go
    assert j == nb and all(f == 0 or f - k >= 2 for k, f in enumerate(fetch))
    return np.asarray([r + (f,) for r, f in zip(rows, fetch)], np.int32).T.copy()


def build(TB=1024, U=3, S=32, NH=12, LO=2, LX=2, R1=128, R2=128, LNR=16, lnhook=((0, 5, 32), (0, 5, 96), (1, 4, 32), (1, 5, 16), (2, 4, 0), (2, 4, 32), (3, 5, 48), (3, 5, 120)), lead=2, DP=1024, batch=True, gh=False,
          orders=((5, 11, 14, 8, 10, 0, 1, 4, 6, 2, 9, 3, 12, 13, 7), (1, 4, 9, 6, 5, 3, 2, 11, 0, 10, 14, 8, 12, 13, 7),
                  (1, 4, 9, 6, 5, 2, 3, 11, 0, 10, 14, 8, 12, 13, 7), (1, 4, 9, 6, 5, 2, 11, 3, 10, 0, 14, 8, 12, 13, 7)), only1=False, rho=0.8, beta=5,
          vmem_mb=127.9, flags=None, nobc=True, its=False):
    M1, M2 = 2 * R1, 2 * R2
    SX = S + LO
    assert TB % M1 == 0 and TB % M2 == 0 and (U * TB // M1) % 2 == 0

    def kernel(tab, x_hbm, dw_ref, w1_hbm, w2_hbm, g_ref, b_ref, o_hbm, h_hbm,
               xbuf, hbuf, ring0, ring1, wc, acc_ref, bias_ref, pin_ref, xsem, x0sem, hsem, osem, wsem, *, nb):
        C, D = w1_hbm.shape
        G = D // 3
        ring = (ring0, ring1)

        rows = lambda k, r, m: pl.ds(pl.multiple_of(k * TB + r, 16), m)
        xslot = lambda s: xbuf.at[pl.ds(pl.multiple_of(s * TB, TB), TB)]
        x_copy = lambda k, s, r, m, sem: pltpu.make_async_copy(
            x_hbm.at[rows(k, r, m)], xslot(s).at[pl.ds(r, m)], sem.at[s])
        x_head = lambda k, s: x_copy(k, s, 0, M1, x0sem)
        x_rest = lambda k, s: x_copy(k, s, M1, TB - M1, xsem)
        x_full = lambda k, s: x_copy(k, s, 0, TB, xsem)
        o_copy = lambda k, s, r=0, m=TB: pltpu.make_async_copy(
            xslot(s).at[pl.ds(r, m)], o_hbm.at[rows(k, r, m)], osem.at[s])
        h_write = lambda k, s: pltpu.make_async_copy(hbuf.at[s], h_hbm.at[k - S], hsem.at[s])
        h_read = lambda k, s, r=0, m=TB: pltpu.make_async_copy(
            h_hbm.at[k - S, pl.ds(r // 2, m // 2)], hbuf.at[s, pl.ds(r // 2, m // 2)], hsem.at[s])
        W0 = S * TB
        w1_copy = [pltpu.make_async_copy(w1_hbm.at[:, pl.ds(q * C, C)], xbuf.at[pl.ds(W0 + q * C, C)], wsem.at[q])
                   for q in range(D // C)]
        w1_tile = lambda r, c: xbuf[pl.ds(W0 + c // C * C + r, 128), pl.ds(c % C, 128)]
        w2_ref = xbuf.at[pl.ds(W0, D)]
        w2_copy = pltpu.make_async_copy(w2_hbm, w2_ref, wsem.at[0])

        def layernorm(xs):
            ds, var = [], None
            for g, xv in enumerate(xs):
                y = xv * dw_ref[...].astype(F32)
                d = y - jnp.sum(y, axis=-1, keepdims=True) * (1.0 / C)
                v = jnp.sum(d * d, axis=-1, keepdims=True)
                ds.append(d)
                if not batch:
                    ds[-1] = d * (lax.rsqrt(v + 1e-5 * C) * (_K * math.sqrt(C)))
                    continue
                v = jnp.broadcast_to(v, (v.shape[0], 128))
                var = v if var is None else jnp.where(lax.broadcasted_iota(jnp.int32, v.shape, 1) == g, v, var)
            if not batch:
                return ds
            inv = lax.rsqrt(var + 1e-5 * C) * (_K * math.sqrt(C))
            return [d * inv[:, g:g + 1] for g, d in enumerate(ds)]

        def normalise(s, r, q, dst):
            n = LNR // 16
            words = [pltpu.bitcast(xslot(s)[pl.ds(r + i * R1 + q + 16 * g, 16), :], U32)
                     for i in range(2) for g in range(n)]
            normed = layernorm([pltpu.unpack_elementwise(w, index=parity, packed_dtype=BF16, unpacked_dtype=F32)
                                for parity in range(2) for w in words])
            combos = []
            for parity in range(2):
                halves = [jnp.concatenate(normed[(2 * parity + i) * n:(2 * parity + i + 1) * n], axis=0)
                          for i in range(2)]
                blk = lambda i, k, halves=halves: halves[i][:, k * 128:(k + 1) * 128]
                lhs = _lhs(blk)
                combos.append({p: blk(*_PLAIN[p]) if p in _PLAIN else lhs(p) for p in _ORDER})
            for p in _ORDER:
                v = pltpu.pack_elementwise([combos[0][p], combos[1][p]], packed_dtype=BF16)
                dst[pl.ds((p * R1 + q) // 2, LNR // 2), :] = pltpu.bitcast(v, U32)

        def expand(src, hv, todo):
            for c in range(0, G, 128):
                done = []

                def prod(p):
                    return jnp.dot(pltpu.bitcast(src[pl.ds(p * R1 // 2, R1 // 2), :], BF16),
                                   pltpu.bitcast(wc[p, pl.ds(c // 2, 64), :], BF16), preferred_element_type=F32)

                def emit(i, j, z):
                    t = jnp.tanh(z * (z * z + _C0))
                    h = z * t + z
                    cols = pl.ds(j * G + c, 128)
                    acc_ref[:, cols] += jnp.sum((h * h).reshape(R1 // 8, 8, 128), axis=0)
                    hv[pl.ds(i * R1 // 2, R1 // 2), cols] = pltpu.bitcast(h.astype(BF16), U32)
                    for tile, out, g in lnhook:
                        if (tile, out) == (c // 128, len(done)):
                            if todo:
                                xbuf[pl.ds(SX * TB, 8), pl.ds(0, 128)] = (h if gh else z)[g:g + 8].astype(BF16)
                                todo.pop(0)()
                    done.append((i, j))

                _combine(prod, emit, orders[c // 128 % len(orders)])

        def project(s, hv, r):
            raw = lambda i, k: pltpu.bitcast(hv[pl.ds((r + i * R2) // 2, R2 // 2), pl.ds(k * G, G)], BF16)
            lhs = _lhs(lambda i, k: raw(i, k).astype(F32))
            xv = xslot(s).at[pl.ds(r, M2)]

            def prod(p):
                a = raw(*_PLAIN[p]) if p in _PLAIN else lhs(p).astype(BF16)
                return jnp.dot(a, pltpu.bitcast(wc[p], BF16), preferred_element_type=F32)

            def emit(i, j, y):
                blk = (pl.ds(i * R2, R2), pl.ds(j * 128, 128))
                res = xv[blk].astype(F32).reshape(R2 // 8, 8, 128) + bias_ref[:, pl.ds(j * 128, 128)]
                xv[blk] = (res.reshape(R2, 128) + y).astype(BF16)

            _combine(prod, emit)

        def rhs(blk):
            for q in range(0, G, 128):
                b = {(k, j): blk(k, j, q) for k in range(3) for j in range(3)}
                for p, terms in enumerate(_RHS):
                    v = None
                    for sign, k, j in sorted(terms, reverse=True):
                        v = b[k, j] if v is None else (v + b[k, j] if sign > 0 else v - b[k, j])
                    wc[p, pl.ds(q // 2, 64), :] = pltpu.bitcast(v.astype(BF16), U32)

        def scoped(f, name):
            if not its:
                return f

            def g(i, c):
                with jax.named_scope(name):
                    return f(i, c)
            return g

        def fetch(t):
            x_head(tab[0, t], tab[1, t]).start()
            x_rest(tab[0, t], tab[1, t]).start()

        with jax.named_scope('pro'):
            for cp in w1_copy:
                cp.start()
            fetch(0)
            acc_ref[...] = jnp.zeros_like(acc_ref)
            for t in range(1, U * LX):
                fetch(t)
            for cp in w1_copy:
                cp.wait()
            rhs(lambda k, j, q: w1_tile(k * 128, j * G + q).astype(F32))
            w2_copy.start()
            x_head(tab[0, 0], tab[1, 0]).wait()
            for q in range(0, R1, LNR):
                normalise(tab[1, 0], 0, q, ring[0])

        def phase1(it, carry):
            t0 = it * U
            blk = [tab[0, t0 + u] for u in range(U + 1)]
            xs = [tab[1, t0 + u] for u in range(U + 1)]
            hs = [tab[2, t0 + u] for u in range(U)]
            for u in range(U):
                x_rest(blk[u], xs[u]).wait()
                if u + 1 < U:
                    x_head(blk[u + 1], xs[u + 1]).wait()
                else:
                    pl.when(t0 + U < nb)(lambda: x_head(blk[U], xs[U]).wait())
                pl.when(tab[3, t0 + u] > 0)(lambda: h_write(S, hs[u]).wait())
            for u in range(U):
                pl.when(t0 + U * LX + u < nb)(functools.partial(fetch, t0 + U * LX + u))
            zero = pl.multiple_of((it >> 20) * 8, 8)

            def piece(n):
                c, q = divmod(n, R1 // LNR)
                u, r = divmod((c + 1) * M1, TB)
                dst = ring[(c + 1) % 2]
                normalise(xs[u], r, q * LNR, dst)
                pin_ref[n] = dst[pl.ds(zero, 8), :]

            todo = [functools.partial(piece, n) for n in range(U * TB // (2 * LNR))]
            for _ in range(lead):
                todo.pop(0)()
            for c in range(U * TB // M1):
                u, r = divmod(c * M1, TB)
                expand(ring[c % 2], hbuf.at[hs[u], pl.ds(r // 2, R1)], todo)
                assert len(todo) <= (U * TB - (c + 1) * M1) // (2 * LNR)
                if r + M1 == TB:
                    pl.when(tab[4, t0 + u] > 0)(lambda: h_write(blk[u], hs[u]).start())
            return carry

        with jax.named_scope('ph1'):
            lax.fori_loop(0, nb // U, scoped(phase1, 'it1'), 0)

        with jax.named_scope('mid'):
            w2_copy.wait()
            nt = D // 128
            row = lambda ref: jnp.concatenate([ref[k:k + 1, :] for k in range(nt)], axis=1)
            g = row(g_ref[...].astype(F32))
            b = jnp.broadcast_to(row(b_ref[...].astype(F32)), (16, D)).astype(BF16)
            bias_ref[...] = jnp.dot(b, w2_ref[...], preferred_element_type=F32)[:8]
            ss = jnp.sum(acc_ref[...], axis=0, keepdims=True) * (1.0 / (_HS * _HS))
            gx = jnp.sqrt(ss + 1e-6)
            nx = gx / (jnp.sum(gx, axis=-1, keepdims=True) * (1.0 / D) + 1e-6)
            sc = (g * nx + 1.0) * (1.0 / _HS)
            col = functools.lru_cache(None)(
                lambda r: jnp.transpose(jnp.broadcast_to(sc[:, r:r + 128], (128, 128))))
            rhs(lambda k, j, q: w2_ref[pl.ds(k * G + q, 128), pl.ds(j * 128, 128)].astype(F32) * col(k * G + q))
            for k in range(S, SX):
                x_full(k, k).start()

        nxt = lambda s, n: jnp.where(s == n - 1, 0, s + 1)

        def phase2(k, carry):
            xs, hs, ps = carry

            @pl.when(k >= S)
            def _():
                h_read(k, hs).wait()
                x_full(k, xs).wait()
            pl.when(k >= LO)(lambda: o_copy(k - LO, ps).wait())
            j = tab[5, k]
            jx, jh = lax.rem(j, SX), lax.rem(j, S)
            pl.when(j >= SX)(lambda: x_full(j, jx).start())
            done = 0
            for r in range(0, TB, M2):
                if not only1:
                    project(xs, hbuf.at[hs], r)
                if r + M2 - done >= DP or r + M2 == TB:
                    pl.when(j > 0)(lambda: h_read(j, jh, done, r + M2 - done).start())
                    o_copy(k, xs, done, r + M2 - done).start()
                    done = r + M2
            return nxt(xs, SX), nxt(hs, S), nxt(ps, SX)

        with jax.named_scope('ph2'):
            lax.fori_loop(0, nb, scoped(phase2, 'it2'), (jnp.int32(0), jnp.int32(0), jnp.int32(S)))
        with jax.named_scope('epi'):
            for k in range(nb - LO, nb):
                o_copy(k, k % SX).wait()

    @jax.jit
    def fn(x, dw, w1, w2, grn_g, grn_b):
        B, H, W, C = x.shape
        D = w1.shape[1]
        N = B * H * W
        nb = N // TB
        assert nb * TB == N and nb % U == 0 and LO * TB >= D
        tab = _plan(nb, S, NH, LO, U, LX, rho, beta)
        vm = pl.BlockSpec(memory_space=pltpu.VMEM)
        hbm = pl.BlockSpec(memory_space=pl.ANY)
        out, _ = pl.pallas_call(
            functools.partial(kernel, nb=nb),
            in_specs=[pl.BlockSpec(memory_space=pltpu.SMEM), hbm, vm, hbm, hbm, vm, vm],
            out_specs=[hbm, hbm],
            out_shape=[jax.ShapeDtypeStruct((N, C), x.dtype),
                       jax.ShapeDtypeStruct((nb - S, TB // 2, D), U32)],
            scratch_shapes=[
                pltpu.VMEM((SX * TB + 64, C), x.dtype),
                pltpu.VMEM((S, TB // 2, D), U32),
                pltpu.VMEM((15 * R1 // 2, 128), U32),
                pltpu.VMEM((15 * R1 // 2, 128), U32),
                pltpu.VMEM((15, D // 6, 128), U32),
                pltpu.VMEM((8, D), F32),
                pltpu.VMEM((8, C), F32),
                pltpu.VMEM((U * TB // (2 * LNR), 8, 128), U32),
                pltpu.SemaphoreType.DMA((SX,)),
                pltpu.SemaphoreType.DMA((SX,)),
                pltpu.SemaphoreType.DMA((S,)),
                pltpu.SemaphoreType.DMA((SX,)),
                pltpu.SemaphoreType.DMA((D // C,)),
            ],
            compiler_params=pltpu.CompilerParams(vmem_limit_bytes=int(vmem_mb * 1024 * 1024), flags=flags,
                                                 disable_bounds_checks=nobc),
            name="slak_block",
        )(tab, x.reshape(N, C), dw.reshape(1, C), w1, w2,
          grn_g.reshape(D // 128, 128), grn_b.reshape(D // 128, 128))
        return out.reshape(B, H, W, C)

    return fn


_fn = build()


def pallas_standalone__modern_conv_block_slak__vision_kernel(x, dw, w1, w2, grn_g, grn_b):
    return _fn(x, dw, w1, w2, grn_g, grn_b)


pallas_standalone__modern_conv_block_slak__vision_kernel = jax.jit(
    pallas_standalone__modern_conv_block_slak__vision_kernel)
```

```python
import functools
import math
import numpy as np
import jax
import jax.numpy as jnp
from jax import lax
import jax.experimental.pallas as pl
import jax.experimental.pallas.tpu as pltpu

_A = math.sqrt(2.0 / math.pi)
_B = _A * 0.044715
_K = _B ** (1.0 / 3.0)
_C0 = _A / _K
_HS = 2.0 * _K
F32, BF16, U32 = jnp.float32, jnp.bfloat16, jnp.uint32

_RHS = (
    ((+1, 1, 0), (-1, 2, 0), (+1, 2, 2)),
    ((+1, 1, 0),),
    ((+1, 0, 0), (+1, 2, 0), (+1, 2, 1)),
    ((+1, 0, 1),),
    ((+1, 1, 0), (+1, 2, 1)),
    ((+1, 0, 0),),
    ((+1, 2, 1),),
    ((+1, 1, 1), (-1, 1, 2), (-1, 2, 1)),
    ((+1, 1, 2),),
    ((+1, 0, 1), (+1, 1, 0), (+1, 1, 1)),
    ((+1, 2, 2),),
    ((+1, 0, 0), (+1, 2, 2)),
    ((+1, 0, 1), (+1, 1, 2)),
    ((-1, 0, 1), (+1, 0, 2), (+1, 2, 2)),
    ((-1, 0, 0), (+1, 0, 2), (+1, 1, 2)),
)


def _lhs(a):
    memo = {}

    def get(r):
        if r not in memo:
            memo[r] = {
                1: lambda: a(1, 1) + a(1, 2),
                3: lambda: a(0, 0) - a(0, 1),
                4: lambda: get(1) - a(0, 1),
                5: lambda: a(0, 0) - a(0, 2),
                6: lambda: get(4) - a(0, 2),
                7: lambda: a(1, 1) - a(0, 1),
                8: lambda: a(1, 0) - a(1, 1),
                10: lambda: get(11) + a(1, 2),
                11: lambda: get(5) - a(1, 0),
                12: lambda: a(1, 0) - a(0, 1),
                13: lambda: a(0, 0) - a(1, 0),
            }[r]()
        return memo[r]
    return get


_PLAIN = {0: (1, 2), 2: (0, 2), 9: (0, 1), 14: (1, 0)}
_ORDER = (1, 4, 9, 6, 5, 2, 3, 11, 0, 10, 14, 8, 12, 13, 7)
_SHARED = {"p": (1, 4), "q": (9, "p"), "s": (11, 5), "t": (14, "s")}
_OUTS = {
    (0, 0): ((+1, 2), (+1, 5), (+1, 6), (+1, "p")),
    (0, 1): ((+1, 3), (+1, "q"), (-1, 6)),
    (1, 0): ((+1, 10), (+1, 1), (-1, 0), (-1, "s")),
    (1, 2): ((+1, 10), (+1, "t"), (-1, 8)),
    (0, 2): ((+1, 13), (+1, 3), (-1, 12), (+1, "t")),
    (1, 1): ((+1, 7), (+1, 12), (-1, 8), (+1, "q")),
}


def _combine(prod, emit, order=_ORDER):
    have, left = {}, dict(_OUTS)
    for r in order:
        have[r] = prod(r)
        for name, (u, v) in _SHARED.items():
            if name not in have and u in have and v in have:
                have[name] = have[u] - have[v]
        for out, terms in list(left.items()):
            if all(key in have for _, key in terms):
                age = list(have)
                terms = sorted(terms, key=lambda term: age.index(term[1]))
                sign, val = terms[0][0], have[terms[0][1]]
                for s, key in terms[1:]:
                    if s == sign:
                        val = val + have[key]
                    else:
                        sign, val = +1, (val - have[key] if sign > 0 else have[key] - val)
                assert sign > 0
                emit(*out, val)
                del left[out]


def _plan(nb, S, NH, U, LX, KR, NR, rho, beta):
    redo = range(KR, KR + NR) if KR < nb else range(0)
    spill = {k: n for n, k in enumerate(k for k in range(S, nb) if k not in redo)}
    keep, stream, order, n = list(range(NH, S)), list(range(S, nb)), [], nb - NH
    for t in range(n):
        due = (t + 1) * (S - NH) // n > t * (S - NH) // n
        order.append(keep.pop() if due else stream.pop())
    order += list(range(NH - 1, -1, -1))
    when = {k: t // U for t, k in enumerate(order)}
    busy = {s: [(when[s] - LX, when[s])] for s in range(NH)}
    tab = np.zeros((10, nb + NR + U * (LX + 1)), np.int32)
    dirty, c = set(), 0
    for t, k in enumerate(order):
        if k < S:
            xs = hs = k
        else:
            lo, hi = t // U - LX, t // U
            xs = next(s for s in busy if all(b < lo or a > hi for a, b in busy[s]))
            busy[xs].append((lo, hi))
            hs, c = c % NH, c + 1
        tab[:7, t] = k, xs, hs, hs in dirty, spill.get(k, -1), t + U * LX < nb, t + 1 < nb
        (dirty.add if k in spill else dirty.discard)(hs)
    assert not dirty
    for u, k in enumerate(redo):
        tab[:7, nb + u] = k, k % (S + 2), k % S, 0, -1, 0, u + 1 < NR
    j, started = S, dict.fromkeys(range(S), -1)
    for k in range(nb):
        clock = k + (NR + 0.5 if k >= KR - NR else 0)
        if j < nb and j - S <= k and (j - S < rho * clock + beta or j - k <= 3):
            assert j - k >= 2 and (j not in redo or k < KR - 1)
            tab[7:9, k] = j, spill.get(j, -1)
            started[j] = k
            j += 1
        tab[9, k] = k in spill
    assert j == nb
    at = max(started[KR], KR - 11) if redo else nb
    held = lambda lo, n: {k % n for k in range(lo, nb) if started[k] < KR or k in redo}
    free_x = next(s for s in range(S + 1) if not {s, s + 1} & held(at - 2, S + 2))
    free_h = next(s for s in range(S) if s not in held(KR - 1, S))
    return tab, (len(spill), at, free_x, free_h)


def build(TB=1024, U=3, S=32, NH=12, LO=2, LX=2, R1=128, R2=128, LNR=16, lnhook=((0, 5, 32), (0, 5, 96), (1, 4, 32), (1, 5, 16), (2, 4, 0), (2, 4, 32), (3, 5, 48), (3, 5, 120)), lead=2, DP=1024, batch=True, gh=False,
          orders=((5, 11, 14, 8, 10, 0, 1, 4, 6, 2, 9, 3, 12, 13, 7), (1, 4, 9, 6, 5, 3, 2, 11, 0, 10, 14, 8, 12, 13, 7),
                  (1, 4, 9, 6, 5, 2, 3, 11, 0, 10, 14, 8, 12, 13, 7), (1, 4, 9, 6, 5, 2, 11, 3, 10, 0, 14, 8, 12, 13, 7)), only1=False, rho=0.8, beta=5, KR=135, RI=1,
          vmem_mb=127.9, flags=None, nobc=True, its=False):
    M1, M2 = 2 * R1, 2 * R2
    SX = S + LO
    assert LO == 2
    assert TB % M1 == 0 and TB % M2 == 0 and (U * TB // M1) % 2 == 0

    def kernel(tab, x_hbm, dw_ref, w1_hbm, w2_hbm, g_ref, b_ref, o_hbm, h_hbm,
               xbuf, hbuf, ring0, ring1, wc, acc_ref, bias_ref, pin_ref, xsem, x0sem, hsem, osem, wsem, *, nb, at, free_x, free_h):
        C, D = w1_hbm.shape
        G = D // 3
        ring = (ring0, ring1)

        rows = lambda k, r, m: pl.ds(pl.multiple_of(k * TB + r, 16), m)
        xslot = lambda s: xbuf.at[pl.ds(pl.multiple_of(s * TB, TB), TB)]
        x_copy = lambda k, s, r, m, sem: pltpu.make_async_copy(
            x_hbm.at[rows(k, r, m)], xslot(s).at[pl.ds(r, m)], sem.at[s])
        x_head = lambda k, s: x_copy(k, s, 0, M1, x0sem)
        x_rest = lambda k, s: x_copy(k, s, M1, TB - M1, xsem)
        x_full = lambda k, s: x_copy(k, s, 0, TB, xsem)
        o_copy = lambda k, s, r=0, m=TB: pltpu.make_async_copy(
            xslot(s).at[pl.ds(r, m)], o_hbm.at[rows(k, r, m)], osem.at[s])
        hslot = lambda s: hbuf.at[pl.ds(pl.multiple_of(s * (TB // 2), TB // 2), TB // 2)]
        h_write = lambda n, s: pltpu.make_async_copy(hslot(s), h_hbm.at[n], hsem.at[s])
        h_read = lambda n, s: pltpu.make_async_copy(h_hbm.at[n], hslot(s), hsem.at[s])
        stage = lambda s: xbuf.at[pl.ds(pl.multiple_of(s * TB, TB), D)]
        w1_copy = lambda s: [pltpu.make_async_copy(w1_hbm.at[:, pl.ds(q * C, C)], stage(s).at[pl.ds(q * C, C)],
                                                   wsem.at[q]) for q in range(D // C)]
        w2_copy = pltpu.make_async_copy(w2_hbm, stage(S), wsem.at[0])
        redo = KR < nb

        def layernorm(xs):
            ds, var = [], None
            for g, xv in enumerate(xs):
                y = xv * dw_ref[...].astype(F32)
                d = y - jnp.sum(y, axis=-1, keepdims=True) * (1.0 / C)
                v = jnp.sum(d * d, axis=-1, keepdims=True)
                ds.append(d)
                if not batch:
                    ds[-1] = d * (lax.rsqrt(v + 1e-5 * C) * (_K * math.sqrt(C)))
                    continue
                v = jnp.broadcast_to(v, (v.shape[0], 128))
                var = v if var is None else jnp.where(lax.broadcasted_iota(jnp.int32, v.shape, 1) == g, v, var)
            if not batch:
                return ds
            inv = lax.rsqrt(var + 1e-5 * C) * (_K * math.sqrt(C))
            return [d * inv[:, g:g + 1] for g, d in enumerate(ds)]

        def normalise(s, r, q, dst):
            n = LNR // 16
            words = [pltpu.bitcast(xslot(s)[pl.ds(r + i * R1 + q + 16 * g, 16), :], U32)
                     for i in range(2) for g in range(n)]
            normed = layernorm([pltpu.unpack_elementwise(w, index=parity, packed_dtype=BF16, unpacked_dtype=F32)
                                for parity in range(2) for w in words])
            combos = []
            for parity in range(2):
                halves = [jnp.concatenate(normed[(2 * parity + i) * n:(2 * parity + i + 1) * n], axis=0)
                          for i in range(2)]
                blk = lambda i, k, halves=halves: halves[i][:, k * 128:(k + 1) * 128]
                lhs = _lhs(blk)
                combos.append({p: blk(*_PLAIN[p]) if p in _PLAIN else lhs(p) for p in _ORDER})
            for p in _ORDER:
                v = pltpu.pack_elementwise([combos[0][p], combos[1][p]], packed_dtype=BF16)
                dst[pl.ds((p * R1 + q) // 2, LNR // 2), :] = pltpu.bitcast(v, U32)

        def expand(src, hv, todo):
            for c in range(0, G, 128):
                done = []

                def prod(p):
                    return jnp.dot(pltpu.bitcast(src[pl.ds(p * R1 // 2, R1 // 2), :], BF16),
                                   pltpu.bitcast(wc[p, pl.ds(c // 2, 64), :], BF16), preferred_element_type=F32)

                def emit(i, j, z):
                    t = jnp.tanh(z * (z * z + _C0))
                    h = z * t + z
                    cols = pl.ds(j * G + c, 128)
                    acc_ref[:, cols] += jnp.sum((h * h).reshape(R1 // 8, 8, 128), axis=0)
                    hv[pl.ds(i * R1 // 2, R1 // 2), cols] = pltpu.bitcast(h.astype(BF16), U32)
                    for tile, out, g in lnhook:
                        if (tile, out) == (c // 128, len(done)):
                            if todo:
                                xbuf[pl.ds(SX * TB, 8), pl.ds(0, 128)] = (h if gh else z)[g:g + 8].astype(BF16)
                                todo.pop(0)()
                    done.append((i, j))

                _combine(prod, emit, orders[c // 128 % len(orders)])

        def project(s, hv, r):
            raw = lambda i, k: pltpu.bitcast(hv[pl.ds((r + i * R2) // 2, R2 // 2), pl.ds(k * G, G)], BF16)
            lhs = _lhs(lambda i, k: raw(i, k).astype(F32))
            xv = xslot(s).at[pl.ds(r, M2)]

            def prod(p):
                a = raw(*_PLAIN[p]) if p in _PLAIN else lhs(p).astype(BF16)
                return jnp.dot(a, pltpu.bitcast(wc[p], BF16), preferred_element_type=F32)

            def emit(i, j, y):
                blk = (pl.ds(i * R2, R2), pl.ds(j * 128, 128))
                res = xv[blk].astype(F32).reshape(R2 // 8, 8, 128) + bias_ref[:, pl.ds(j * 128, 128)]
                xv[blk] = (res.reshape(R2, 128) + y).astype(BF16)

            _combine(prod, emit)

        def rhs(blk):
            for q in range(0, G, 128):
                b = {(k, j): blk(k, j, q) for k in range(3) for j in range(3)}
                for p, terms in enumerate(_RHS):
                    v = None
                    for sign, k, j in sorted(terms, reverse=True):
                        v = b[k, j] if v is None else (v + b[k, j] if sign > 0 else v - b[k, j])
                    wc[p, pl.ds(q // 2, 64), :] = pltpu.bitcast(v.astype(BF16), U32)

        def scoped(f, name):
            if not its:
                return f

            def g(i, c):
                with jax.named_scope(name):
                    return f(i, c)
            return g

        def fetch(t):
            x_head(tab[0, t], tab[1, t]).start()
            x_rest(tab[0, t], tab[1, t]).start()

        def prepare(t, ws):
            for cp in w1_copy(ws):
                cp.wait()
            rhs(lambda k, j, q: stage(ws)[pl.ds((j * G + q) // C * C + k * 128, 128),
                                          pl.ds((j * G + q) % C, 128)].astype(F32))
            x_head(tab[0, t], tab[1, t]).wait()
            for q in range(0, R1, LNR):
                normalise(tab[1, t], 0, q, ring[0])

        def phase1(it, carry):
            t0 = it * U
            blk = [tab[0, t0 + u] for u in range(U + 1)]
            xs = [tab[1, t0 + u] for u in range(U + 1)]
            xs[U] = jnp.where(tab[6, t0 + U - 1] > 0, xs[U], xs[0])
            hs = [tab[2, t0 + u] for u in range(U)]
            for u in range(U):
                x_rest(blk[u], xs[u]).wait()
                if u + 1 < U:
                    x_head(blk[u + 1], xs[u + 1]).wait()
                else:
                    pl.when(tab[6, t0 + u] > 0)(lambda: x_head(blk[U], xs[U]).wait())
                pl.when(tab[3, t0 + u] > 0)(lambda: h_write(0, hs[u]).wait())
            for u in range(U):
                pl.when(tab[5, t0 + u] > 0)(functools.partial(fetch, t0 + U * LX + u))
            zero = pl.multiple_of((it >> 20) * 8, 8)

            def piece(n):
                c, q = divmod(n, R1 // LNR)
                u, r = divmod((c + 1) * M1, TB)
                dst = ring[(c + 1) % 2]
                normalise(xs[u], r, q * LNR, dst)
                pin_ref[n] = dst[pl.ds(zero, 8), :]

            todo = [functools.partial(piece, n) for n in range(U * TB // (2 * LNR))]
            for _ in range(lead):
                todo.pop(0)()
            for c in range(U * TB // M1):
                u, r = divmod(c * M1, TB)
                expand(ring[c % 2], hslot(hs[u]).at[pl.ds(r // 2, R1)], todo)
                assert len(todo) <= (U * TB - (c + 1) * M1) // (2 * LNR)
                if r + M1 == TB:
                    pl.when(tab[4, t0 + u] >= 0)(lambda: h_write(tab[4, t0 + u], hs[u]).start())
            return carry

        def rescale():
            w2_copy.wait()
            w2_ref = stage(S)
            nt = D // 128
            row = lambda ref: jnp.concatenate([ref[k:k + 1, :] for k in range(nt)], axis=1)
            g = row(g_ref[...].astype(F32))
            b = jnp.broadcast_to(row(b_ref[...].astype(F32)), (16, D)).astype(BF16)
            bias_ref[...] = jnp.dot(b, w2_ref[...], preferred_element_type=F32)[:8]
            ss = jnp.sum(acc_ref[...], axis=0, keepdims=True) * (1.0 / (_HS * _HS))
            gx = jnp.sqrt(ss + 1e-6)
            nx = gx / (jnp.sum(gx, axis=-1, keepdims=True) * (1.0 / D) + 1e-6)
            sc = (g * nx + 1.0) * (1.0 / _HS)
            col = functools.lru_cache(None)(
                lambda r: jnp.transpose(jnp.broadcast_to(sc[:, r:r + 128], (128, 128))))
            rhs(lambda k, j, q: w2_ref[pl.ds(k * G + q, 128), pl.ds(j * 128, 128)].astype(F32) * col(k * G + q))
            for k in range(S, SX):
                x_full(k, k).start()

        nxt = lambda s, n: jnp.where(s == n - 1, 0, s + 1)

        def phase2(k, carry):
            xs, hs, ps = carry

            @pl.when(tab[9, k] > 0)
            def _():
                h_read(0, hs).wait()
                x_full(k, xs).wait()
            pl.when(k >= LO)(lambda: o_copy(k - LO, ps).wait())
            j, n = tab[7, k], tab[8, k]
            jx, jh = lax.rem(j, SX), lax.rem(j, S)
            pl.when(jnp.logical_and(j >= SX, n >= 0))(lambda: x_full(j, jx).start())
            if redo:
                @pl.when(n < 0)
                def _():
                    x_head(j, jx).start()
                    x_rest(j, jx).start()

                @pl.when(k == at)
                def _():
                    for cp in w1_copy(free_x):
                        cp.start()
            for r in range(0, TB, M2):
                if not only1:
                    project(xs, hslot(hs), r)
            pl.when(jnp.logical_and(j > 0, n >= 0))(lambda: h_read(n, jh).start())
            o_copy(k, xs).start()
            return nxt(xs, SX), nxt(hs, S), nxt(ps, SX)

        for cp in w1_copy(S):
            cp.start()
        acc_ref[...] = jnp.zeros_like(acc_ref)
        for t in range(U * LX):
            fetch(t)

        def shelve(back):
            for n in range(15 * G // 128):
                p, q = divmod(n, G // 128)
                r, c = divmod(n, D // 128)
                here = wc.at[p, pl.ds(q * 64, 64)]
                there = hbuf.at[pl.ds(free_h * (TB // 2) + r * 64, 64), pl.ds(c * 128, 128)]
                if back:
                    here[...] = there[...]
                else:
                    there[...] = here[...]

        def sweep(rnd, carry):
            first = rnd == 0
            pick = lambda a, b: jnp.where(first, a, b)
            with jax.named_scope('pro'):
                if redo:
                    pl.when(rnd > 0)(functools.partial(shelve, False))
                prepare(pick(0, nb), pick(S, free_x))
                pl.when(first)(w2_copy.start)
            with jax.named_scope('ph1'):
                lax.fori_loop(pick(0, nb // U), pick(nb // U, nb // U + RI), scoped(phase1, 'it1'), 0)
            with jax.named_scope('mid'):
                pl.when(first)(rescale)
                if redo:
                    pl.when(rnd > 0)(functools.partial(shelve, True))
            with jax.named_scope('ph2'):
                return lax.fori_loop(pick(0, KR), pick(min(KR, nb), nb), scoped(phase2, 'it2'), carry)

        lax.fori_loop(0, 2 if redo else 1, sweep, (jnp.int32(0), jnp.int32(0), jnp.int32(S)))
        with jax.named_scope('epi'):
            for k in range(nb - LO, nb):
                o_copy(k, k % SX).wait()

    @jax.jit
    def fn(x, dw, w1, w2, grn_g, grn_b):
        B, H, W, C = x.shape
        D = w1.shape[1]
        N = B * H * W
        nb = N // TB
        assert nb * TB == N and nb % U == 0 and LO * TB >= D
        tab, (spilled, at, free_x, free_h) = _plan(nb, S, NH, U, LX, KR, RI * U, rho, beta)
        vm = pl.BlockSpec(memory_space=pltpu.VMEM)
        hbm = pl.BlockSpec(memory_space=pl.ANY)
        out, _ = pl.pallas_call(
            functools.partial(kernel, nb=nb, at=at, free_x=free_x, free_h=free_h),
            in_specs=[pl.BlockSpec(memory_space=pltpu.SMEM), hbm, vm, hbm, hbm, vm, vm],
            out_specs=[hbm, hbm],
            out_shape=[jax.ShapeDtypeStruct((N, C), x.dtype),
                       jax.ShapeDtypeStruct((spilled, TB // 2, D), U32)],
            scratch_shapes=[
                pltpu.VMEM((SX * TB + 64, C), x.dtype),
                pltpu.VMEM((S * TB // 2, D), U32),
                pltpu.VMEM((15 * R1 // 2, 128), U32),
                pltpu.VMEM((15 * R1 // 2, 128), U32),
                pltpu.VMEM((15, D // 6, 128), U32),
                pltpu.VMEM((8, D), F32),
                pltpu.VMEM((8, C), F32),
                pltpu.VMEM((U * TB // (2 * LNR), 8, 128), U32),
                pltpu.SemaphoreType.DMA((SX,)),
                pltpu.SemaphoreType.DMA((SX,)),
                pltpu.SemaphoreType.DMA((S,)),
                pltpu.SemaphoreType.DMA((SX,)),
                pltpu.SemaphoreType.DMA((D // C,)),
            ],
            compiler_params=pltpu.CompilerParams(vmem_limit_bytes=int(vmem_mb * 1024 * 1024), flags=flags,
                                                 disable_bounds_checks=nobc),
            name="slak_block",
        )(tab, x.reshape(N, C), dw.reshape(1, C), w1, w2,
          grn_g.reshape(D // 128, 128), grn_b.reshape(D // 128, 128))
        return out.reshape(B, H, W, C)

    return fn


_fn = build(KR=105,beta=4.5)


def pallas_standalone__modern_conv_block_slak__vision_kernel(x, dw, w1, w2, grn_g, grn_b):
    return _fn(x, dw, w1, w2, grn_g, grn_b)


pallas_standalone__modern_conv_block_slak__vision_kernel = jax.jit(
    pallas_standalone__modern_conv_block_slak__vision_kernel)
```

```python
import functools
import math
import numpy as np
import jax
import jax.numpy as jnp
from jax import lax
import jax.experimental.pallas as pl
import jax.experimental.pallas.tpu as pltpu

_A = math.sqrt(2.0 / math.pi)
_B = _A * 0.044715
_K = _B ** (1.0 / 3.0)
_C0 = _A / _K
_HS = 2.0 * _K
F32, BF16, U32 = jnp.float32, jnp.bfloat16, jnp.uint32

_RHS = (
    ((+1, 1, 0), (-1, 2, 0), (+1, 2, 2)),
    ((+1, 1, 0),),
    ((+1, 0, 0), (+1, 2, 0), (+1, 2, 1)),
    ((+1, 0, 1),),
    ((+1, 1, 0), (+1, 2, 1)),
    ((+1, 0, 0),),
    ((+1, 2, 1),),
    ((+1, 1, 1), (-1, 1, 2), (-1, 2, 1)),
    ((+1, 1, 2),),
    ((+1, 0, 1), (+1, 1, 0), (+1, 1, 1)),
    ((+1, 2, 2),),
    ((+1, 0, 0), (+1, 2, 2)),
    ((+1, 0, 1), (+1, 1, 2)),
    ((-1, 0, 1), (+1, 0, 2), (+1, 2, 2)),
    ((-1, 0, 0), (+1, 0, 2), (+1, 1, 2)),
)


def _lhs(a):
    memo = {}

    def get(r):
        if r not in memo:
            memo[r] = {
                1: lambda: a(1, 1) + a(1, 2),
                3: lambda: a(0, 0) - a(0, 1),
                4: lambda: get(1) - a(0, 1),
                5: lambda: a(0, 0) - a(0, 2),
                6: lambda: get(4) - a(0, 2),
                7: lambda: a(1, 1) - a(0, 1),
                8: lambda: a(1, 0) - a(1, 1),
                10: lambda: get(11) + a(1, 2),
                11: lambda: get(5) - a(1, 0),
                12: lambda: a(1, 0) - a(0, 1),
                13: lambda: a(0, 0) - a(1, 0),
            }[r]()
        return memo[r]
    return get


_PLAIN = {0: (1, 2), 2: (0, 2), 9: (0, 1), 14: (1, 0)}
_ORDER = (1, 4, 9, 6, 5, 2, 3, 11, 0, 10, 14, 8, 12, 13, 7)
_SHARED = {"p": (1, 4), "q": (9, "p"), "s": (11, 5), "t": (14, "s")}
_OUTS = {
    (0, 0): ((+1, 2), (+1, 5), (+1, 6), (+1, "p")),
    (0, 1): ((+1, 3), (+1, "q"), (-1, 6)),
    (1, 0): ((+1, 10), (+1, 1), (-1, 0), (-1, "s")),
    (1, 2): ((+1, 10), (+1, "t"), (-1, 8)),
    (0, 2): ((+1, 13), (+1, 3), (-1, 12), (+1, "t")),
    (1, 1): ((+1, 7), (+1, 12), (-1, 8), (+1, "q")),
}


def _combine(prod, emit, order=_ORDER):
    have, left = {}, dict(_OUTS)
    for r in order:
        have[r] = prod(r)
        for name, (u, v) in _SHARED.items():
            if name not in have and u in have and v in have:
                have[name] = have[u] - have[v]
        for out, terms in list(left.items()):
            if all(key in have for _, key in terms):
                age = list(have)
                terms = sorted(terms, key=lambda term: age.index(term[1]))
                sign, val = terms[0][0], have[terms[0][1]]
                for s, key in terms[1:]:
                    if s == sign:
                        val = val + have[key]
                    else:
                        sign, val = +1, (val - have[key] if sign > 0 else have[key] - val)
                assert sign > 0
                emit(*out, val)
                del left[out]


def _plan(nb, S, NH, U, V, LX, KR, NR, rho, beta):
    redo = range(KR, KR + NR) if KR < nb else range(0)
    spill = {k: n for n, k in enumerate(k for k in range(S, nb) if k not in redo)}
    keep, stream, order, n = list(range(NH, S)), list(range(S, nb)), [], nb - NH
    for t in range(n):
        due = (t + 1) * (S - NH) // n > t * (S - NH) // n
        order.append(keep.pop() if due else stream.pop())
    order += list(range(NH - 1, -1, -1))
    when = {k: t // U for t, k in enumerate(order)}
    busy = {s: [(when[s] - LX, when[s])] for s in range(NH)}
    tab = np.zeros((12, nb + NR + U * (LX + 1)), np.int32)
    dirty, c = set(), 0
    for t, k in enumerate(order):
        if k < S:
            xs = hs = k
        else:
            lo, hi = t // U - LX, t // U
            xs = next(s for s in busy if all(b < lo or a > hi for a, b in busy[s]))
            busy[xs].append((lo, hi))
            hs, c = c % NH, c + 1
        tab[:7, t] = k, xs, hs, hs in dirty, spill.get(k, -1), t + U * LX < nb, t + 1 < nb
        (dirty.add if k in spill else dirty.discard)(hs)
    assert not dirty
    for u, k in enumerate(redo):
        tab[:7, nb + u] = k, k % (S + 2), k % S, 0, -1, 0, u + 1 < NR
    j, i, started = S, S + 2, dict.fromkeys(range(S), -1)
    for k in range(nb):
        clock = k + (NR + 0.5 if k >= KR - NR else 0)
        if j < nb and j - S <= k and (j - S < rho * clock + beta or j - k <= 2 * V):
            tab[7:9, k] = j, spill.get(j, -1)
            started[j] = k
            j += 1
        if i < j and i - (S + 2) < k // V * V - V:
            assert i >= k // V * V + V and (i not in redo or k < KR - 1)
            tab[10:12, k] = i, i in redo and (i - KR) % U == 0
            i += 1
        tab[9, k] = k in spill
    assert i == nb and j == nb and started[S] == 0 and KR % V == 0 and nb % V == 0
    at = max(started[KR], KR - 11) if redo else nb
    held = lambda lo, n: {k % n for k in range(lo, nb) if started[k] < KR or k in redo}
    free_x = next(s for s in range(S + 1) if not {s, s + 1} & held(at // V * V - V, S + 2))
    free_h = next(s for s in range(S) if s not in held(KR - 1, S))
    return tab, (len(spill), at, free_x, free_h)


def build(TB=1024, U=3, S=32, NH=12, LO=2, LX=2, R1=128, R2=128, LNR=16, lnhook=((0, 5, 32), (0, 5, 96), (1, 4, 32), (1, 5, 16), (2, 4, 0), (2, 4, 32), (3, 5, 48), (3, 5, 120)), lead=2, DP=1024, batch=True, gh=False,
          orders=((5, 11, 14, 8, 10, 0, 1, 4, 6, 2, 9, 3, 12, 13, 7), (1, 4, 9, 6, 5, 3, 2, 11, 0, 10, 14, 8, 12, 13, 7),
                  (1, 4, 9, 6, 5, 2, 3, 11, 0, 10, 14, 8, 12, 13, 7), (1, 4, 9, 6, 5, 2, 11, 3, 10, 0, 14, 8, 12, 13, 7)), only1=False, rho=0.8, beta=4, KR=105, fine=512, V=1, RI=1,
          vmem_mb=127.9, flags=None, nobc=True, its=False):
    M1, M2 = 2 * R1, 2 * R2
    SX = S + LO
    assert LO == 2
    assert TB % M1 == 0 and TB % M2 == 0 and (U * TB // M1) % 2 == 0

    def kernel(tab_hbm, x_hbm, dw_hbm, w1_hbm, w2_hbm, g_hbm, b_hbm, o_hbm, h_hbm,
               xbuf, hbuf, ring0, ring1, wc, acc_ref, bias_ref, pin_ref, dw_ref, g_ref, b_ref, tab, xsem, x0sem, hsem, osem, wsem, ssem, *, nb, lead_in, at, free_x, free_h):
        C, D = w1_hbm.shape
        G = D // 3
        ring = (ring0, ring1)

        rows = lambda k, r, m: pl.ds(pl.multiple_of(k * TB + r, 16), m)
        xslot = lambda s: xbuf.at[pl.ds(pl.multiple_of(s * TB, TB), TB)]
        x_copy = lambda k, s, r, m, sem: pltpu.make_async_copy(
            x_hbm.at[rows(k, r, m)], xslot(s).at[pl.ds(r, m)], sem.at[s])
        x_head = lambda k, s: x_copy(k, s, 0, M1, x0sem)
        x_rest = lambda k, s: x_copy(k, s, M1, TB - M1, xsem)
        x_full = lambda k, s: x_copy(k, s, 0, TB, xsem)
        o_copy = lambda k, s, r=0, m=TB: pltpu.make_async_copy(
            xslot(s).at[pl.ds(r, m)], o_hbm.at[rows(k, r, m)], osem.at[s])
        hslot = lambda s: hbuf.at[pl.ds(pl.multiple_of(s * (TB // 2), TB // 2), TB // 2)]
        h_write = lambda n, s: pltpu.make_async_copy(hslot(s), h_hbm.at[n], hsem.at[s])
        h_read = lambda n, s, r=0, m=TB: pltpu.make_async_copy(
            h_hbm.at[n, pl.ds(r // 2, m // 2)], hslot(s).at[pl.ds(r // 2, m // 2)], hsem.at[s])
        stage = lambda s: xbuf.at[pl.ds(pl.multiple_of(s * TB, TB), D)]
        w1_copy = lambda s: [pltpu.make_async_copy(w1_hbm.at[:, pl.ds(q * C, C)], stage(s).at[pl.ds(q * C, C)],
                                                   wsem.at[q]) for q in range(D // C)]
        w2_copy = pltpu.make_async_copy(w2_hbm, stage(S), wsem.at[0])
        redo = KR < nb

        def layernorm(xs):
            ds, var = [], None
            for g, xv in enumerate(xs):
                y = xv * dw_ref[...].astype(F32)
                d = y - jnp.sum(y, axis=-1, keepdims=True) * (1.0 / C)
                v = jnp.sum(d * d, axis=-1, keepdims=True)
                ds.append(d)
                if not batch:
                    ds[-1] = d * (lax.rsqrt(v + 1e-5 * C) * (_K * math.sqrt(C)))
                    continue
                v = jnp.broadcast_to(v, (v.shape[0], 128))
                var = v if var is None else jnp.where(lax.broadcasted_iota(jnp.int32, v.shape, 1) == g, v, var)
            if not batch:
                return ds
            inv = lax.rsqrt(var + 1e-5 * C) * (_K * math.sqrt(C))
            return [d * inv[:, g:g + 1] for g, d in enumerate(ds)]

        def normalise(s, r, q, dst):
            n = LNR // 16
            words = [pltpu.bitcast(xslot(s)[pl.ds(r + i * R1 + q + 16 * g, 16), :], U32)
                     for i in range(2) for g in range(n)]
            normed = layernorm([pltpu.unpack_elementwise(w, index=parity, packed_dtype=BF16, unpacked_dtype=F32)
                                for parity in range(2) for w in words])
            combos = []
            for parity in range(2):
                halves = [jnp.concatenate(normed[(2 * parity + i) * n:(2 * parity + i + 1) * n], axis=0)
                          for i in range(2)]
                blk = lambda i, k, halves=halves: halves[i][:, k * 128:(k + 1) * 128]
                lhs = _lhs(blk)
                combos.append({p: blk(*_PLAIN[p]) if p in _PLAIN else lhs(p) for p in _ORDER})
            for p in _ORDER:
                v = pltpu.pack_elementwise([combos[0][p], combos[1][p]], packed_dtype=BF16)
                dst[pl.ds((p * R1 + q) // 2, LNR // 2), :] = pltpu.bitcast(v, U32)

        def expand(src, hv, todo):
            for c in range(0, G, 128):
                done = []

                def prod(p):
                    return jnp.dot(pltpu.bitcast(src[pl.ds(p * R1 // 2, R1 // 2), :], BF16),
                                   pltpu.bitcast(wc[p, pl.ds(c // 2, 64), :], BF16), preferred_element_type=F32)

                def emit(i, j, z):
                    t = jnp.tanh(z * (z * z + _C0))
                    h = z * t + z
                    cols = pl.ds(j * G + c, 128)
                    acc_ref[:, cols] += jnp.sum((h * h).reshape(R1 // 8, 8, 128), axis=0)
                    hv[pl.ds(i * R1 // 2, R1 // 2), cols] = pltpu.bitcast(h.astype(BF16), U32)
                    for tile, out, g in lnhook:
                        if (tile, out) == (c // 128, len(done)):
                            if todo:
                                xbuf[pl.ds(SX * TB, 8), pl.ds(0, 128)] = (h if gh else z)[g:g + 8].astype(BF16)
                                todo.pop(0)()
                    done.append((i, j))

                _combine(prod, emit, orders[c // 128 % len(orders)])

        def project(s, hv, r):
            raw = lambda i, k: pltpu.bitcast(hv[pl.ds((r + i * R2) // 2, R2 // 2), pl.ds(k * G, G)], BF16)
            lhs = _lhs(lambda i, k: raw(i, k).astype(F32))
            xv = xslot(s).at[pl.ds(r, M2)]

            def prod(p):
                a = raw(*_PLAIN[p]) if p in _PLAIN else lhs(p).astype(BF16)
                return jnp.dot(a, pltpu.bitcast(wc[p], BF16), preferred_element_type=F32)

            def emit(i, j, y):
                blk = (pl.ds(i * R2, R2), pl.ds(j * 128, 128))
                res = xv[blk].astype(F32).reshape(R2 // 8, 8, 128) + bias_ref[:, pl.ds(j * 128, 128)]
                xv[blk] = (res.reshape(R2, 128) + y).astype(BF16)

            _combine(prod, emit)

        def rhs(blk):
            for q in range(0, G, 128):
                b = {(k, j): blk(k, j, q) for k in range(3) for j in range(3)}
                for p, terms in enumerate(_RHS):
                    v = None
                    for sign, k, j in sorted(terms, reverse=True):
                        v = b[k, j] if v is None else (v + b[k, j] if sign > 0 else v - b[k, j])
                    wc[p, pl.ds(q // 2, 64), :] = pltpu.bitcast(v.astype(BF16), U32)

        def scoped(f, name):
            if not its:
                return f

            def g(i, c):
                with jax.named_scope(name):
                    return f(i, c)
            return g

        def fetch(k, s, split):
            for cp in (x_head(k, s), x_rest(k, s)) if split else (x_full(k, s),):
                cp.start()

        def prepare(t, ws):
            for cp in w1_copy(ws):
                cp.wait()
            rhs(lambda k, j, q: stage(ws)[pl.ds((j * G + q) // C * C + k * 128, 128),
                                          pl.ds((j * G + q) % C, 128)].astype(F32))
            x_head(tab[0, t], tab[1, t]).wait()
            for q in range(0, R1, LNR):
                normalise(tab[1, t], 0, q, ring[0])

        def lookup(t0):
            return ([tab[1, t0 + u] for u in range(U + 1)], [tab[2, t0 + u] for u in range(U)],
                    [tab[3, t0 + u] for u in range(U)], tab[6, t0 + U - 1])

        def phase1(it, carry):
            t0 = it * U
            xs, hs, busy, more = carry
            x_rest(0, xs[0]).wait()
            for u in range(1, U):
                x_full(0, xs[u]).wait()
            pl.when(more > 0)(lambda: x_head(0, xs[U]).wait())
            xs = xs[:U] + [jnp.where(more > 0, xs[U], xs[0])]
            for u in range(U):
                pl.when(busy[u] > 0)(lambda: h_write(0, hs[u]).wait())
            for u in range(U):
                t = t0 + U * LX + u
                pl.when(tab[5, t0 + u] > 0)(lambda: fetch(tab[0, t], tab[1, t], u == 0))
            zero = pl.multiple_of((it >> 20) * 8, 8)

            def piece(n):
                c, q = divmod(n, R1 // LNR)
                u, r = divmod((c + 1) * M1, TB)
                dst = ring[(c + 1) % 2]
                normalise(xs[u], r, q * LNR, dst)
                pin_ref[n] = dst[pl.ds(zero, 8), :]

            todo = [functools.partial(piece, n) for n in range(U * TB // (2 * LNR))]
            for _ in range(lead):
                todo.pop(0)()
            for c in range(U * TB // M1):
                u, r = divmod(c * M1, TB)
                expand(ring[c % 2], hslot(hs[u]).at[pl.ds(r // 2, R1)], todo)
                assert len(todo) <= (U * TB - (c + 1) * M1) // (2 * LNR)
                if r + M1 == TB:
                    pl.when(tab[4, t0 + u] >= 0)(lambda: h_write(tab[4, t0 + u], hs[u]).start())
            return lookup(t0 + U)

        def rescale():
            w2_copy.wait()
            w2_ref = stage(S)
            nt = D // 128
            row = lambda ref: jnp.concatenate([ref[k:k + 1, :] for k in range(nt)], axis=1)
            g = row(g_ref[...].astype(F32))
            b = jnp.broadcast_to(row(b_ref[...].astype(F32)), (16, D)).astype(BF16)
            bias_ref[...] = jnp.dot(b, w2_ref[...], preferred_element_type=F32)[:8]
            ss = jnp.sum(acc_ref[...], axis=0, keepdims=True) * (1.0 / (_HS * _HS))
            gx = jnp.sqrt(ss + 1e-6)
            nx = gx / (jnp.sum(gx, axis=-1, keepdims=True) * (1.0 / D) + 1e-6)
            sc = (g * nx + 1.0) * (1.0 / _HS)
            col = functools.lru_cache(None)(
                lambda r: jnp.transpose(jnp.broadcast_to(sc[:, r:r + 128], (128, 128))))
            rhs(lambda k, j, q: w2_ref[pl.ds(k * G + q, 128), pl.ds(j * 128, 128)].astype(F32) * col(k * G + q))
            for k in range(S, SX):
                x_full(k, k).start()

        nxt = lambda s, n: jnp.where(s == n - 1, 0, s + 1)

        def phase2(it, carry):
            xs, hs, ps = [[c] for c in carry[:3]]
            for v in range(V):
                xs.append(nxt(xs[v], SX))
                hs.append(nxt(hs[v], S))
                ps.append(nxt(ps[v], SX))
            for v in range(V):
                k = it * V + v

                @pl.when(carry[3][v] > 0)
                def _():
                    h_read(0, hs[v]).wait()
                    x_full(k, xs[v]).wait()
                pl.when(k >= 2 * V)(lambda: o_copy(k - 2 * V, ps[v]).wait())
            for v in range(V):
                k = it * V + v
                i, j, n = tab[10, k], tab[7, k], tab[8, k]
                pl.when(jnp.logical_and(i > 0, tab[11, k] == 0))(lambda: x_full(i, lax.rem(i, SX)).start())
                if redo:
                    pl.when(tab[11, k] > 0)(lambda: fetch(i, lax.rem(i, SX), True))

                    if v == at % V:
                        @pl.when(k == at)
                        def _():
                            for cp in w1_copy(free_x):
                                cp.start()
                opening, closing = fine and v == 0, fine and v == V - 1
                for r in range(0, TB, M2):
                    if not only1:
                        project(xs[v], hslot(hs[v]), r)
                    if opening and (r + M2) % fine == 0:
                        pl.when(k == 0)(lambda: h_read(0, 0, r + M2 - fine, fine).start())
                    if closing and (r + M2) % fine == 0:
                        pl.when(k == nb - 1)(lambda: o_copy(nb - 1, (nb - 1) % SX, r + M2 - fine, fine).start())
                pl.when(jnp.logical_and(j > (S if opening else 0), n >= 0))(lambda: h_read(n, lax.rem(j, S)).start())
                pl.when(k < nb - (1 if closing else 0))(lambda: o_copy(k, xs[v]).start())
            return xs[V], hs[V], ps[V], [tab[9, it * V + V + v] for v in range(V)]

        small = [pltpu.make_async_copy(src, dst, ssem.at[n]) for n, (src, dst) in enumerate(
            ((tab_hbm, tab), (dw_hbm, dw_ref), (g_hbm, g_ref), (b_hbm, b_ref)))]
        for cp in small + w1_copy(S):
            cp.start()
        acc_ref[...] = jnp.zeros_like(acc_ref)
        for cp in small:
            cp.wait()
        for t, (k, s) in enumerate(lead_in):
            fetch(k, s, t % U == 0)

        def shelve(back):
            for n in range(15 * G // 128):
                p, q = divmod(n, G // 128)
                r, c = divmod(n, D // 128)
                here = wc.at[p, pl.ds(q * 64, 64)]
                there = hbuf.at[pl.ds(free_h * (TB // 2) + r * 64, 64), pl.ds(c * 128, 128)]
                if back:
                    here[...] = there[...]
                else:
                    there[...] = here[...]

        def sweep(rnd, carry):
            first = rnd == 0
            pick = lambda a, b: jnp.where(first, a, b)
            with jax.named_scope('pro'):
                if redo:
                    pl.when(rnd > 0)(functools.partial(shelve, False))
                prepare(pick(0, nb), pick(S, free_x))
                pl.when(first)(w2_copy.start)
            with jax.named_scope('ph1'):
                lax.fori_loop(pick(0, nb // U), pick(nb // U, nb // U + RI), scoped(phase1, 'it1'), lookup(pick(0, nb)))
            with jax.named_scope('mid'):
                pl.when(first)(rescale)
                if redo:
                    pl.when(rnd > 0)(functools.partial(shelve, True))
            with jax.named_scope('ph2'):
                return lax.fori_loop(pick(0, KR // V), pick(min(KR, nb) // V, nb // V), scoped(phase2, 'it2'), carry)

        lax.fori_loop(0, 2 if redo else 1, sweep, (jnp.int32(0), jnp.int32(0), jnp.int32(SX - 2 * V), [jnp.int32(0)] * V))
        with jax.named_scope('epi'):
            for k in range(nb - 2 * V, nb):
                o_copy(k, k % SX).wait()

    @jax.jit
    def fn(x, dw, w1, w2, grn_g, grn_b):
        B, H, W, C = x.shape
        D = w1.shape[1]
        N = B * H * W
        nb = N // TB
        assert nb * TB == N and nb % U == 0 and LO * TB >= D
        tab, (spilled, at, free_x, free_h) = _plan(nb, S, NH, U, V, LX, KR, RI * U, rho, beta)
        hbm = pl.BlockSpec(memory_space=pl.ANY)
        out, _ = pl.pallas_call(
            functools.partial(kernel, nb=nb, lead_in=[(int(k), int(s)) for k, s in tab[:2, :U * LX].T], at=at, free_x=free_x, free_h=free_h),
            in_specs=[hbm] * 7,
            out_specs=[hbm, hbm],
            out_shape=[jax.ShapeDtypeStruct((N, C), x.dtype),
                       jax.ShapeDtypeStruct((spilled, TB // 2, D), U32)],
            scratch_shapes=[
                pltpu.VMEM((SX * TB + 64, C), x.dtype),
                pltpu.VMEM((S * TB // 2, D), U32),
                pltpu.VMEM((15 * R1 // 2, 128), U32),
                pltpu.VMEM((15 * R1 // 2, 128), U32),
                pltpu.VMEM((15, D // 6, 128), U32),
                pltpu.VMEM((8, D), F32),
                pltpu.VMEM((8, C), F32),
                pltpu.VMEM((U * TB // (2 * LNR), 8, 128), U32),
                pltpu.VMEM((1, C), dw.dtype),
                pltpu.VMEM((D // 128, 128), grn_g.dtype),
                pltpu.VMEM((D // 128, 128), grn_b.dtype),
                pltpu.SMEM(tab.shape, jnp.int32),
                pltpu.SemaphoreType.DMA((SX,)),
                pltpu.SemaphoreType.DMA((SX,)),
                pltpu.SemaphoreType.DMA((S,)),
                pltpu.SemaphoreType.DMA((SX,)),
                pltpu.SemaphoreType.DMA((D // C,)),
                pltpu.SemaphoreType.DMA((4,)),
            ],
            compiler_params=pltpu.CompilerParams(vmem_limit_bytes=int(vmem_mb * 1024 * 1024), flags=flags,
                                                 disable_bounds_checks=nobc),
            name="slak_block",
        )(tab, x.reshape(N, C), dw.reshape(1, C), w1, w2,
          grn_g.reshape(D // 128, 128), grn_b.reshape(D // 128, 128))
        return out.reshape(B, H, W, C)

    return fn


_fn = build(lead=2,batch=True,gh=False,lnhook=((0, 5, 64), (0, 5, 96), (1, 4, 64), (1, 5, 0), (2, 3, 0), (2, 4, 32), (3, 5, 16), (3, 5, 120)),orders=((5, 11, 14, 8, 10, 0, 1, 4, 6, 2, 9, 3, 12, 13, 7), (1, 4, 9, 6, 2, 5, 3, 11, 0, 10, 14, 8, 12, 13, 7), (1, 9, 4, 6, 5, 3, 2, 11, 0, 10, 14, 8, 12, 13, 7), (1, 4, 9, 6, 5, 2, 3, 11, 0, 10, 14, 8, 12, 13, 7)))


def pallas_standalone__modern_conv_block_slak__vision_kernel(x, dw, w1, w2, grn_g, grn_b):
    return _fn(x, dw, w1, w2, grn_g, grn_b)


pallas_standalone__modern_conv_block_slak__vision_kernel = jax.jit(
    pallas_standalone__modern_conv_block_slak__vision_kernel)
```

```python
import functools
import math

import jax
import jax.experimental.pallas as pl
import jax.experimental.pallas.tpu as pltpu
import jax.numpy as jnp
import numpy as np
from jax import lax

F32, BF16, U32 = jnp.float32, jnp.bfloat16, jnp.uint32

_A = math.sqrt(2.0 / math.pi)
_K = (_A * 0.044715) ** (1.0 / 3.0)
_C0 = _A / _K
_HS = 2.0 * _K

R = 128
TB = 1024
U = 3
S = 32
NH = 12
LX = 2
KR = 105
PACE = (0.8, 4)
LNR = 16

_RHS = (
    ((+1, 2, 2), (+1, 1, 0), (-1, 2, 0)),
    ((+1, 1, 0),),
    ((+1, 2, 1), (+1, 2, 0), (+1, 0, 0)),
    ((+1, 0, 1),),
    ((+1, 2, 1), (+1, 1, 0)),
    ((+1, 0, 0),),
    ((+1, 2, 1),),
    ((+1, 1, 1), (-1, 2, 1), (-1, 1, 2)),
    ((+1, 1, 2),),
    ((+1, 1, 1), (+1, 1, 0), (+1, 0, 1)),
    ((+1, 2, 2),),
    ((+1, 2, 2), (+1, 0, 0)),
    ((+1, 1, 2), (+1, 0, 1)),
    ((+1, 2, 2), (+1, 0, 2), (-1, 0, 1)),
    ((+1, 1, 2), (+1, 0, 2), (-1, 0, 0)),
)
_PLAIN = {0: (1, 2), 2: (0, 2), 9: (0, 1), 14: (1, 0)}
_SHARED = {"p": (1, 4), "q": (9, "p"), "s": (11, 5), "t": (14, "s")}
_OUTS = {
    (0, 0): ((+1, 2), (+1, 5), (+1, 6), (+1, "p")),
    (0, 1): ((+1, 3), (+1, "q"), (-1, 6)),
    (1, 0): ((+1, 10), (+1, 1), (-1, 0), (-1, "s")),
    (1, 2): ((+1, 10), (+1, "t"), (-1, 8)),
    (0, 2): ((+1, 13), (+1, 3), (-1, 12), (+1, "t")),
    (1, 1): ((+1, 7), (+1, 12), (-1, 8), (+1, "q")),
}
_ORDER = (1, 4, 9, 6, 5, 2, 3, 11, 0, 10, 14, 8, 12, 13, 7)
_TILE_ORDER = (
    (5, 11, 14, 8, 10, 0, 1, 4, 6, 2, 9, 3, 12, 13, 7),
    (1, 4, 9, 6, 2, 5, 3, 11, 0, 10, 14, 8, 12, 13, 7),
    (1, 9, 4, 6, 5, 3, 2, 11, 0, 10, 14, 8, 12, 13, 7),
    (1, 4, 9, 6, 5, 2, 3, 11, 0, 10, 14, 8, 12, 13, 7),
)
_GATES = ((0, 5, 64), (0, 5, 96), (1, 4, 64), (1, 5, 0), (2, 3, 0), (2, 4, 32), (3, 5, 16), (3, 5, 120))
_LEAD = 2


def _lhs(a):
    @functools.lru_cache(None)
    def get(r):
        return {
            1: lambda: a(1, 1) + a(1, 2),
            3: lambda: a(0, 0) - a(0, 1),
            4: lambda: get(1) - a(0, 1),
            5: lambda: a(0, 0) - a(0, 2),
            6: lambda: get(4) - a(0, 2),
            7: lambda: a(1, 1) - a(0, 1),
            8: lambda: a(1, 0) - a(1, 1),
            10: lambda: get(11) + a(1, 2),
            11: lambda: get(5) - a(1, 0),
            12: lambda: a(1, 0) - a(0, 1),
            13: lambda: a(0, 0) - a(1, 0),
        }[r]()
    return get


def _combine(prod, emit, order):
    have, left = {}, dict(_OUTS)
    for r in order:
        have[r] = prod(r)
        for name, (u, v) in _SHARED.items():
            if name not in have and u in have and v in have:
                have[name] = have[u] - have[v]
        for out, terms in list(left.items()):
            if all(key in have for _, key in terms):
                age = list(have)
                terms = sorted(terms, key=lambda term: age.index(term[1]))
                sign, val = terms[0][0], have[terms[0][1]]
                for s, key in terms[1:]:
                    if s == sign:
                        val = val + have[key]
                    else:
                        sign, val = +1, (val - have[key] if sign > 0 else have[key] - val)
                assert sign > 0
                emit(*out, val)
                del left[out]


BLK, XS, HS, BUSY, PUT, AHEAD, MORE, H_BLK, GET, FAR, X_BLK, SPLIT = range(12)


def _plan(nb):
    redo = range(KR, KR + U)
    place = {k: n for n, k in enumerate(k for k in range(S, nb) if k not in redo)}
    keep, stream, order, n = list(range(NH, S)), list(range(S, nb)), [], nb - NH
    for t in range(n):
        due = (t + 1) * (S - NH) // n > t * (S - NH) // n
        order.append(keep.pop() if due else stream.pop())
    order += list(range(NH - 1, -1, -1))
    turn = {k: t // U for t, k in enumerate(order)}
    taken = {s: [(turn[s] - LX, turn[s])] for s in range(NH)}
    tab = np.zeros((12, nb + U * (LX + 2)), np.int32)
    dirty, c = [False] * S, 0
    for t, k in enumerate(order):
        if k < S:
            xs = hs = k
        else:
            lo, hi = t // U - LX, t // U
            xs = next(s for s in range(NH) if all(b < lo or a > hi for a, b in taken[s]))
            taken[xs].append((lo, hi))
            hs, c = c % NH, c + 1
        tab[:7, t] = k, xs, hs, dirty[hs], place.get(k, -1), t + U * LX < nb, t + 1 < nb
        dirty[hs] = k in place
    assert not any(dirty)
    for u, k in enumerate(redo):
        tab[:7, nb + u] = k, k % (S + 2), k % S, 0, -1, 0, u + 1 < U
    j, i, started = S, S + 2, dict.fromkeys(range(S), -1)
    for k in range(nb):
        clock = k + (U + 0.5 if k >= KR - U else 0)
        if j < nb and j - S <= k and (j - S < PACE[0] * clock + PACE[1] or j - k <= 2):
            tab[[H_BLK, GET], k] = j, place.get(j, -1)
            started[j] = k
            j += 1
        if i < j and i - (S + 2) <= k - 2:
            assert i > k and (i not in redo or k < KR)
            tab[[X_BLK, SPLIT], k] = i, i == KR
            i += 1
        tab[FAR, k] = k in place
    assert i == j == nb and started[S] == 0
    at = max(started[KR], KR - 11)
    held = lambda lo, n: [k % n for k in range(lo, nb) if started[k] < KR or k in redo]
    free_x = next(s for s in range(S + 1) if s not in held(at - 1, S + 2) and s + 1 not in held(at - 1, S + 2))
    free_h = next(s for s in range(S) if s not in held(KR - 1, S))
    return tab, len(place), (at, free_x, free_h)


def _kernel(tab_hbm, x_hbm, dw_hbm, w1_hbm, w2_hbm, g_hbm, b_hbm, o_hbm, h_hbm,
            xbuf, hbuf, ring0, ring1, wc, acc_ref, bias_ref, pin_ref, dw_ref, g_ref, b_ref, tab,
            xsem, x0sem, hsem, osem, wsem, ssem, *, nb, lead_in, borrow):
    C, D = w1_hbm.shape
    G, M, SX = D // 3, 2 * R, S + 2
    ring = (ring0, ring1)
    at, free_x, free_h = borrow

    rows = lambda k, r, m: pl.ds(pl.multiple_of(k * TB + r, 16), m)
    xslot = lambda s: xbuf.at[pl.ds(pl.multiple_of(s * TB, TB), TB)]
    hslot = lambda s: hbuf.at[pl.ds(pl.multiple_of(s * (TB // 2), TB // 2), TB // 2)]
    x_copy = lambda k, s, r, m, sem: pltpu.make_async_copy(
        x_hbm.at[rows(k, r, m)], xslot(s).at[pl.ds(r, m)], sem.at[s])
    x_head = lambda k, s: x_copy(k, s, 0, M, x0sem)
    x_rest = lambda k, s: x_copy(k, s, M, TB - M, xsem)
    x_full = lambda k, s: x_copy(k, s, 0, TB, xsem)
    o_copy = lambda k, s, r=0, m=TB: pltpu.make_async_copy(
        xslot(s).at[pl.ds(r, m)], o_hbm.at[rows(k, r, m)], osem.at[s])
    h_write = lambda n, s: pltpu.make_async_copy(hslot(s), h_hbm.at[n], hsem.at[s])
    h_read = lambda n, s, r=0, m=TB: pltpu.make_async_copy(
        h_hbm.at[n, pl.ds(r // 2, m // 2)], hslot(s).at[pl.ds(r // 2, m // 2)], hsem.at[s])
    stage = lambda s: xbuf.at[pl.ds(pl.multiple_of(s * TB, TB), D)]
    w1_copy = lambda s: [pltpu.make_async_copy(w1_hbm.at[:, pl.ds(q * C, C)], stage(s).at[pl.ds(q * C, C)],
                                               wsem.at[q]) for q in range(D // C)]
    w2_copy = pltpu.make_async_copy(w2_hbm, stage(S), wsem.at[0])

    def fetch(k, s, split):
        for cp in (x_head(k, s), x_rest(k, s)) if split else (x_full(k, s),):
            cp.start()

    def layernorm(xs):
        ds, var = [], None
        for g, xv in enumerate(xs):
            y = xv * dw_ref[...].astype(F32)
            d = y - jnp.sum(y, axis=-1, keepdims=True) * (1.0 / C)
            v = jnp.broadcast_to(jnp.sum(d * d, axis=-1, keepdims=True), (d.shape[0], 128))
            ds.append(d)
            var = v if var is None else jnp.where(lax.broadcasted_iota(jnp.int32, v.shape, 1) == g, v, var)
        inv = lax.rsqrt(var + 1e-5 * C) * (_K * math.sqrt(C))
        return [d * inv[:, g:g + 1] for g, d in enumerate(ds)]

    def normalise(s, r, q, dst):
        words = [pltpu.bitcast(xslot(s)[pl.ds(r + i * R + q, LNR), :], U32) for i in range(2)]
        normed = layernorm([pltpu.unpack_elementwise(w, index=parity, packed_dtype=BF16, unpacked_dtype=F32)
                            for parity in range(2) for w in words])
        combos = []
        for parity in range(2):
            blk = lambda i, k, parity=parity: normed[2 * parity + i][:, k * 128:(k + 1) * 128]
            lhs = _lhs(blk)
            combos.append({p: blk(*_PLAIN[p]) if p in _PLAIN else lhs(p) for p in _ORDER})
        for p in _ORDER:
            v = pltpu.pack_elementwise([combos[0][p], combos[1][p]], packed_dtype=BF16)
            dst[pl.ds((p * R + q) // 2, LNR // 2), :] = pltpu.bitcast(v, U32)

    def expand(src, hv, todo):
        for tile in range(G // 128):
            done = []

            def prod(p):
                return jnp.dot(pltpu.bitcast(src[pl.ds(p * R // 2, R // 2), :], BF16),
                               pltpu.bitcast(wc[p, pl.ds(tile * 64, 64), :], BF16), preferred_element_type=F32)

            def emit(i, j, z):
                h = z * jnp.tanh(z * (z * z + _C0)) + z
                cols = pl.ds(j * G + tile * 128, 128)
                acc_ref[:, cols] += jnp.sum((h * h).reshape(R // 8, 8, 128), axis=0)
                hv[pl.ds(i * R // 2, R // 2), cols] = pltpu.bitcast(h.astype(BF16), U32)
                for gate in _GATES:
                    if gate[:2] == (tile, len(done)) and todo:
                        xbuf[pl.ds(SX * TB, 8), pl.ds(0, 128)] = z[gate[2]:gate[2] + 8].astype(BF16)
                        todo.pop(0)()
                done.append((i, j))

            _combine(prod, emit, _TILE_ORDER[tile])

    def project(s, hv, r):
        raw = lambda i, k: pltpu.bitcast(hv[pl.ds((r + i * R) // 2, R // 2), pl.ds(k * G, G)], BF16)
        lhs = _lhs(lambda i, k: raw(i, k).astype(F32))
        xv = xslot(s).at[pl.ds(r, M)]

        def prod(p):
            a = raw(*_PLAIN[p]) if p in _PLAIN else lhs(p).astype(BF16)
            return jnp.dot(a, pltpu.bitcast(wc[p], BF16), preferred_element_type=F32)

        def emit(i, j, y):
            blk = (pl.ds(i * R, R), pl.ds(j * 128, 128))
            res = xv[blk].astype(F32).reshape(R // 8, 8, 128) + bias_ref[:, pl.ds(j * 128, 128)]
            xv[blk] = (res.reshape(R, 128) + y).astype(BF16)

        _combine(prod, emit, _ORDER)

    def rhs(blk):
        for q in range(0, G, 128):
            b = {(k, j): blk(k, j, q) for k in range(3) for j in range(3)}
            for p, terms in enumerate(_RHS):
                v = b[terms[0][1:]]
                for sign, k, j in terms[1:]:
                    v = v + b[k, j] if sign > 0 else v - b[k, j]
                wc[p, pl.ds(q // 2, 64), :] = pltpu.bitcast(v.astype(BF16), U32)

    def prepare(t, ws):
        for cp in w1_copy(ws):
            cp.wait()
        rhs(lambda k, j, q: stage(ws)[pl.ds((j * G + q) // C * C + k * 128, 128),
                                      pl.ds((j * G + q) % C, 128)].astype(F32))
        x_head(0, tab[XS, t]).wait()
        for q in range(0, R, LNR):
            normalise(tab[XS, t], 0, q, ring[0])

    def lookup(t):
        return ([tab[XS, t + u] for u in range(U + 1)], [tab[HS, t + u] for u in range(U)],
                [tab[BUSY, t + u] for u in range(U)], tab[MORE, t + U - 1])

    def phase1(it, carry):
        t0 = it * U
        xs, hs, busy, more = carry
        x_rest(0, xs[0]).wait()
        for u in range(1, U):
            x_full(0, xs[u]).wait()
        pl.when(more > 0)(lambda: x_head(0, xs[U]).wait())
        xs = xs[:U] + [jnp.where(more > 0, xs[U], xs[0])]
        for u in range(U):
            pl.when(busy[u] > 0)(lambda: h_write(0, hs[u]).wait())
        for u in range(U):
            t = t0 + U * LX + u
            pl.when(tab[AHEAD, t0 + u] > 0)(lambda: fetch(tab[BLK, t], tab[XS, t], u == 0))
        zero = pl.multiple_of((it >> 20) * 8, 8)

        def piece(n):
            c, q = divmod(n, R // LNR)
            u, r = divmod((c + 1) * M, TB)
            dst = ring[(c + 1) % 2]
            normalise(xs[u], r, q * LNR, dst)
            pin_ref[n] = dst[pl.ds(zero, 8), :]

        todo = [functools.partial(piece, n) for n in range(U * TB // (2 * LNR))]
        for _ in range(_LEAD):
            todo.pop(0)()
        for c in range(U * TB // M):
            u, r = divmod(c * M, TB)
            expand(ring[c % 2], hslot(hs[u]).at[pl.ds(r // 2, R)], todo)
            left = (U * TB - (c + 1) * M) // (2 * LNR)
            assert left - R // LNR <= len(todo) <= left
            if r + M == TB:
                pl.when(tab[PUT, t0 + u] >= 0)(lambda: h_write(tab[PUT, t0 + u], hs[u]).start())
        return lookup(t0 + U)

    def rescale():
        w2_copy.wait()
        w2 = stage(S)
        row = lambda v: jnp.concatenate([v[k:k + 1, :] for k in range(D // 128)], axis=1)
        b = jnp.broadcast_to(row(b_ref[...].astype(F32)), (16, D)).astype(BF16)
        bias_ref[...] = jnp.dot(b, w2[...], preferred_element_type=F32)[:8]
        gx = jnp.sqrt(jnp.sum(acc_ref[...], axis=0, keepdims=True) * (1.0 / (_HS * _HS)) + 1e-6)
        nx = gx / (jnp.sum(gx, axis=-1, keepdims=True) * (1.0 / D) + 1e-6)
        scale = (row(g_ref[...].astype(F32)) * nx + 1.0) * (1.0 / _HS)
        col = functools.lru_cache(None)(lambda r: jnp.transpose(jnp.broadcast_to(scale[:, r:r + 128], (128, 128))))
        rhs(lambda k, j, q: w2[pl.ds(k * G + q, 128), pl.ds(j * 128, 128)].astype(F32) * col(k * G + q))
        for k in range(S, SX):
            x_full(k, k).start()

    nxt = lambda s, n: jnp.where(s == n - 1, 0, s + 1)

    def phase2(k, carry):
        xs, hs, ps, far = carry

        @pl.when(far > 0)
        def _():
            h_read(0, hs).wait()
            x_full(0, xs).wait()
        pl.when(k >= 2)(lambda: o_copy(0, ps).wait())
        i, j, n = tab[X_BLK, k], tab[H_BLK, k], tab[GET, k]
        pl.when(jnp.logical_and(i > 0, tab[SPLIT, k] == 0))(lambda: fetch(i, lax.rem(i, SX), False))
        pl.when(tab[SPLIT, k] > 0)(lambda: fetch(i, lax.rem(i, SX), True))

        @pl.when(k == at)
        def _():
            for cp in w1_copy(free_x):
                cp.start()
        half = TB // 2
        for r in range(0, TB, M):
            project(xs, hslot(hs), r)
            if (r + M) % half == 0:
                pl.when(k == 0)(lambda: h_read(0, 0, r + M - half, half).start())
                pl.when(k == nb - 1)(lambda: o_copy(nb - 1, (nb - 1) % SX, r + M - half, half).start())
        pl.when(jnp.logical_and(j > S, n >= 0))(lambda: h_read(n, lax.rem(j, S)).start())
        pl.when(k < nb - 1)(lambda: o_copy(k, xs).start())
        return nxt(xs, SX), nxt(hs, S), nxt(ps, SX), tab[FAR, k + 1]

    def shelve(back):
        for n in range(15 * G // 128):
            p, q = divmod(n, G // 128)
            r, c = divmod(n, D // 128)
            here = wc.at[p, pl.ds(q * 64, 64)]
            there = (pl.ds(free_h * (TB // 2) + r * 64, 64), pl.ds(c * 128, 128))
            if back:
                here[...] = hbuf[there]
            else:
                hbuf[there] = here[...]

    small = [pltpu.make_async_copy(src, dst, ssem.at[n]) for n, (src, dst) in enumerate(
        ((tab_hbm, tab), (dw_hbm, dw_ref), (g_hbm, g_ref), (b_hbm, b_ref)))]
    for cp in small + w1_copy(S):
        cp.start()
    acc_ref[...] = jnp.zeros_like(acc_ref)
    for cp in small:
        cp.wait()
    for t, (k, s) in enumerate(lead_in):
        fetch(k, s, t % U == 0)

    def sweep(rnd, carry):
        first = rnd == 0
        pick = lambda a, b: jnp.where(first, a, b)
        pl.when(rnd > 0)(functools.partial(shelve, False))
        prepare(pick(0, nb), pick(S, free_x))
        pl.when(first)(lambda: w2_copy.start())
        lax.fori_loop(pick(0, nb // U), pick(nb // U, nb // U + 1), phase1, lookup(pick(0, nb)))
        pl.when(first)(rescale)
        pl.when(rnd > 0)(functools.partial(shelve, True))
        return lax.fori_loop(pick(0, KR), pick(KR, nb), phase2, carry)

    lax.fori_loop(0, 2, sweep, (jnp.int32(0), jnp.int32(0), jnp.int32(S), jnp.int32(0)))
    for k in range(nb - 2, nb):
        o_copy(k, k % SX).wait()


@jax.jit
def pallas_standalone__modern_conv_block_slak__vision_kernel(
    x: jax.Array,
    dw: jax.Array,
    w1: jax.Array,
    w2: jax.Array,
    grn_g: jax.Array,
    grn_b: jax.Array,
):
    B, H, W, C = x.shape
    D = w1.shape[1]
    N = H * W
    assert B == 1 and dw.shape == (1, 1, C) and (C, D) == (384, 1536) and N % (U * TB) == 0
    nb = N // TB
    tab, parked, borrow = _plan(nb)
    hbm = pl.BlockSpec(memory_space=pl.ANY)
    out, _ = pl.pallas_call(
        functools.partial(_kernel, nb=nb, borrow=borrow,
                          lead_in=[(int(k), int(s)) for k, s in tab[[BLK, XS], :U * LX].T]),
        in_specs=[hbm] * 7,
        out_specs=[hbm, hbm],
        out_shape=[jax.ShapeDtypeStruct((N, C), BF16), jax.ShapeDtypeStruct((parked, TB // 2, D), U32)],
        scratch_shapes=[
            pltpu.VMEM(((S + 2) * TB + 64, C), BF16),
            pltpu.VMEM((S * TB // 2, D), U32),
            pltpu.VMEM((15 * R // 2, 128), U32),
            pltpu.VMEM((15 * R // 2, 128), U32),
            pltpu.VMEM((15, D // 6, 128), U32),
            pltpu.VMEM((8, D), F32),
            pltpu.VMEM((8, C), F32),
            pltpu.VMEM((U * TB // (2 * LNR), 8, 128), U32),
            pltpu.VMEM((1, C), dw.dtype),
            pltpu.VMEM((D // 128, 128), grn_g.dtype),
            pltpu.VMEM((D // 128, 128), grn_b.dtype),
            pltpu.SMEM(tab.shape, jnp.int32),
            pltpu.SemaphoreType.DMA((S + 2,)),
            pltpu.SemaphoreType.DMA((S + 2,)),
            pltpu.SemaphoreType.DMA((S,)),
            pltpu.SemaphoreType.DMA((S + 2,)),
            pltpu.SemaphoreType.DMA((D // C,)),
            pltpu.SemaphoreType.DMA((4,)),
        ],
        compiler_params=pltpu.CompilerParams(vmem_limit_bytes=int(127.9 * 2 ** 20), disable_bounds_checks=True),
        name="slak_block",
    )(tab, x.reshape(N, C).astype(BF16), dw.reshape(1, C), w1.astype(BF16), w2.astype(BF16),
      grn_g.reshape(D // 128, 128), grn_b.reshape(D // 128, 128))
    return out.reshape(B, H, W, C).astype(x.dtype)
```

```python
import functools
import math

import jax
import jax.experimental.pallas as pl
import jax.experimental.pallas.tpu as pltpu
import jax.numpy as jnp
import numpy as np
from jax import lax

F32, BF16, U32 = jnp.float32, jnp.bfloat16, jnp.uint32

_A = math.sqrt(2.0 / math.pi)
_K = (_A * 0.044715) ** (1.0 / 3.0)
_C0 = _A / _K
_HS = 2.0 * _K

R = 128
TB = 1024
U = 3
S = 32
NH = 12
LX = 2
KR = 105
PACE = (0.8, 4)
LNR = 16

_RHS = (
    ((+1, 2, 2), (+1, 1, 0), (-1, 2, 0)),
    ((+1, 1, 0),),
    ((+1, 2, 1), (+1, 2, 0), (+1, 0, 0)),
    ((+1, 0, 1),),
    ((+1, 2, 1), (+1, 1, 0)),
    ((+1, 0, 0),),
    ((+1, 2, 1),),
    ((+1, 1, 1), (-1, 2, 1), (-1, 1, 2)),
    ((+1, 1, 2),),
    ((+1, 1, 1), (+1, 1, 0), (+1, 0, 1)),
    ((+1, 2, 2),),
    ((+1, 2, 2), (+1, 0, 0)),
    ((+1, 1, 2), (+1, 0, 1)),
    ((+1, 2, 2), (+1, 0, 2), (-1, 0, 1)),
    ((+1, 1, 2), (+1, 0, 2), (-1, 0, 0)),
)
_PLAIN = {0: (1, 2), 2: (0, 2), 9: (0, 1), 14: (1, 0)}
_SHARED = {"p": (1, 4), "q": (9, "p"), "s": (11, 5), "t": (14, "s")}
_OUTS = {
    (0, 0): ((+1, 2), (+1, 5), (+1, 6), (+1, "p")),
    (0, 1): ((+1, 3), (+1, "q"), (-1, 6)),
    (1, 0): ((+1, 10), (+1, 1), (-1, 0), (-1, "s")),
    (1, 2): ((+1, 10), (+1, "t"), (-1, 8)),
    (0, 2): ((+1, 13), (+1, 3), (-1, 12), (+1, "t")),
    (1, 1): ((+1, 7), (+1, 12), (-1, 8), (+1, "q")),
}
_ORDER = (1, 4, 9, 6, 5, 2, 3, 11, 0, 10, 14, 8, 12, 13, 7)
_TILE_ORDER = (
    (5, 11, 14, 8, 10, 0, 1, 4, 6, 2, 9, 3, 12, 13, 7),
    (1, 4, 9, 6, 2, 5, 3, 11, 0, 10, 14, 8, 12, 13, 7),
    (1, 9, 4, 6, 5, 3, 2, 11, 0, 10, 14, 8, 12, 13, 7),
    (1, 4, 9, 6, 5, 2, 3, 11, 0, 10, 14, 8, 12, 13, 7),
)
_GATES = ((0, 5, 64), (0, 5, 96), (1, 4, 64), (1, 5, 0), (2, 3, 0), (2, 4, 32), (3, 5, 16), (3, 5, 120))
_LEAD = 2


def _lhs(a):
    @functools.lru_cache(None)
    def get(r):
        return {
            1: lambda: a(1, 1) + a(1, 2),
            3: lambda: a(0, 0) - a(0, 1),
            4: lambda: get(1) - a(0, 1),
            5: lambda: a(0, 0) - a(0, 2),
            6: lambda: get(4) - a(0, 2),
            7: lambda: a(1, 1) - a(0, 1),
            8: lambda: a(1, 0) - a(1, 1),
            10: lambda: get(11) + a(1, 2),
            11: lambda: get(5) - a(1, 0),
            12: lambda: a(1, 0) - a(0, 1),
            13: lambda: a(0, 0) - a(1, 0),
        }[r]()
    return get


def _combine(prod, emit, order):
    have, left = {}, dict(_OUTS)
    for r in order:
        have[r] = prod(r)
        for name, (u, v) in _SHARED.items():
            if name not in have and u in have and v in have:
                have[name] = have[u] - have[v]
        for out, terms in list(left.items()):
            if all(key in have for _, key in terms):
                age = list(have)
                terms = sorted(terms, key=lambda term: age.index(term[1]))
                sign, val = terms[0][0], have[terms[0][1]]
                for s, key in terms[1:]:
                    if s == sign:
                        val = val + have[key]
                    else:
                        sign, val = +1, (val - have[key] if sign > 0 else have[key] - val)
                assert sign > 0
                emit(*out, val)
                del left[out]


BLK, XS, HS, BUSY, PUT, AHEAD, MORE, H_BLK, GET, FAR, X_BLK, SPLIT = range(12)


def _plan(nb):
    redo = range(KR, KR + U)
    place = {k: n for n, k in enumerate(k for k in range(S, nb) if k not in redo)}
    keep, stream, order, n = list(range(NH, S)), list(range(S, nb)), [], nb - NH
    for t in range(n):
        due = (t + 1) * (S - NH) // n > t * (S - NH) // n
        order.append(keep.pop() if due else stream.pop())
    order += list(range(NH - 1, -1, -1))
    turn = {k: t // U for t, k in enumerate(order)}
    taken = {s: [(turn[s] - LX, turn[s])] for s in range(NH)}
    tab = np.zeros((12, nb + U * (LX + 2)), np.int32)
    dirty, c = [False] * S, 0
    for t, k in enumerate(order):
        if k < S:
            xs = hs = k
        else:
            lo, hi = t // U - LX, t // U
            xs = next(s for s in range(NH) if all(b < lo or a > hi for a, b in taken[s]))
            taken[xs].append((lo, hi))
            hs, c = c % NH, c + 1
        tab[:7, t] = k, xs, hs, dirty[hs], place.get(k, -1), t + U * LX < nb, t + 1 < nb
        dirty[hs] = k in place
    assert not any(dirty)
    for u, k in enumerate(redo):
        tab[:7, nb + u] = k, k % (S + 2), k % S, 0, -1, 0, u + 1 < U
    j, i, started = S, S + 2, dict.fromkeys(range(S), -1)
    for k in range(nb):
        clock = k + (U + 0.5 if k >= KR - U else 0)
        if j < nb and j - S <= k and (j - S < PACE[0] * clock + PACE[1] or j - k <= 2):
            tab[[H_BLK, GET], k] = j, place.get(j, -1)
            started[j] = k
            j += 1
        if i < j and i - (S + 2) <= k - 2:
            assert i > k and (i not in redo or k < KR)
            tab[[X_BLK, SPLIT], k] = i, i == KR
            i += 1
        tab[FAR, k] = k in place
    assert i == j == nb and started[S] == 0
    at = max(started[KR], KR - 11)
    held = lambda lo, n: [k % n for k in range(lo, nb) if started[k] < KR or k in redo]
    free_x = next(s for s in range(S + 1) if s not in held(at - 1, S + 2) and s + 1 not in held(at - 1, S + 2))
    free_h = next(s for s in range(S) if s not in held(KR - 1, S))
    return tab, len(place), (at, free_x, free_h)


def _kernel(tab_hbm, x_hbm, dw_hbm, w1_hbm, w2_hbm, g_hbm, b_hbm, o_hbm, h_hbm,
            xbuf, hbuf, ring0, ring1, wc, acc_ref, bias_ref, pin_ref, dw_ref, g_ref, b_ref, tab,
            xsem, x0sem, hsem, osem, wsem, ssem, *, nb, lead_in, borrow):
    C, D = w1_hbm.shape
    G, M, SX = D // 3, 2 * R, S + 2
    ring = (ring0, ring1)
    at, free_x, free_h = borrow

    rows = lambda k, r, m: pl.ds(pl.multiple_of(k * TB + r, 16), m)
    xslot = lambda s: xbuf.at[pl.ds(pl.multiple_of(s * TB, TB), TB)]
    hslot = lambda s: hbuf.at[pl.ds(pl.multiple_of(s * (TB // 2), TB // 2), TB // 2)]
    x_copy = lambda k, s, r, m, sem: pltpu.make_async_copy(
        x_hbm.at[rows(k, r, m)], xslot(s).at[pl.ds(r, m)], sem.at[s])
    x_head = lambda k, s: x_copy(k, s, 0, M, x0sem)
    x_rest = lambda k, s: x_copy(k, s, M, TB - M, xsem)
    x_full = lambda k, s: x_copy(k, s, 0, TB, xsem)
    o_copy = lambda k, s, r=0, m=TB: pltpu.make_async_copy(
        xslot(s).at[pl.ds(r, m)], o_hbm.at[rows(k, r, m)], osem.at[s])
    h_write = lambda n, s: pltpu.make_async_copy(hslot(s), h_hbm.at[n], hsem.at[s])
    h_read = lambda n, s, r=0, m=TB: pltpu.make_async_copy(
        h_hbm.at[n, pl.ds(r // 2, m // 2)], hslot(s).at[pl.ds(r // 2, m // 2)], hsem.at[s])
    stage = lambda s: xbuf.at[pl.ds(pl.multiple_of(s * TB, TB), D)]
    w1_copy = lambda s: [pltpu.make_async_copy(w1_hbm.at[:, pl.ds(q * C, C)], stage(s).at[pl.ds(q * C, C)],
                                               wsem.at[q]) for q in range(D // C)]
    w2_copy = pltpu.make_async_copy(w2_hbm, stage(S), wsem.at[0])

    def fetch(k, s, split):
        for cp in (x_head(k, s), x_rest(k, s)) if split else (x_full(k, s),):
            cp.start()

    def layernorm(xs):
        ds, var = [], None
        for g, xv in enumerate(xs):
            y = xv * dw_ref[...].astype(F32)
            d = y - jnp.sum(y, axis=-1, keepdims=True) * (1.0 / C)
            v = jnp.broadcast_to(jnp.sum(d * d, axis=-1, keepdims=True), (d.shape[0], 128))
            ds.append(d)
            var = v if var is None else jnp.where(lax.broadcasted_iota(jnp.int32, v.shape, 1) == g, v, var)
        inv = lax.rsqrt(var + 1e-5 * C) * (_K * math.sqrt(C))
        return [d * inv[:, g:g + 1] for g, d in enumerate(ds)]

    def normalise(s, r, q, dst):
        n = LNR // 8
        xs = [xslot(s)[pl.ds(r + i * R + q, LNR), :].astype(F32) for i in range(2)]
        normed = layernorm([v[8 * g:8 * g + 8] for v in xs for g in range(n)])
        halves = [jnp.concatenate(normed[i * n:(i + 1) * n], axis=0) for i in range(2)]
        blk = lambda i, k: halves[i][:, k * 128:(k + 1) * 128]
        lhs = _lhs(blk)
        for p in _ORDER:
            v = blk(*_PLAIN[p]) if p in _PLAIN else lhs(p)
            dst[pl.ds(q // 2, LNR // 2), pl.ds(p * 128, 128)] = pltpu.bitcast(v.astype(BF16), U32)

    def expand(src, hv, todo):
        for tile in range(G // 128):
            done = []

            def prod(p):
                return jnp.dot(pltpu.bitcast(src[:, pl.ds(p * 128, 128)], BF16),
                               pltpu.bitcast(wc[p, pl.ds(tile * 64, 64), :], BF16), preferred_element_type=F32)

            def emit(i, j, z):
                h = z * jnp.tanh(z * (z * z + _C0)) + z
                cols = pl.ds(j * G + tile * 128, 128)
                acc_ref[:, cols] += jnp.sum((h * h).reshape(R // 8, 8, 128), axis=0)
                hv[pl.ds(i * R // 2, R // 2), cols] = pltpu.bitcast(h.astype(BF16), U32)
                for gate in _GATES:
                    if gate[:2] == (tile, len(done)) and todo:
                        xbuf[pl.ds(SX * TB, 8), pl.ds(0, 128)] = z[gate[2]:gate[2] + 8].astype(BF16)
                        todo.pop(0)()
                done.append((i, j))

            _combine(prod, emit, _TILE_ORDER[tile])

    def project(s, hv, r):
        raw = lambda i, k: pltpu.bitcast(hv[pl.ds((r + i * R) // 2, R // 2), pl.ds(k * G, G)], BF16)
        lhs = _lhs(lambda i, k: raw(i, k).astype(F32))
        xv = xslot(s).at[pl.ds(r, M)]

        def prod(p):
            a = raw(*_PLAIN[p]) if p in _PLAIN else lhs(p).astype(BF16)
            return jnp.dot(a, pltpu.bitcast(wc[p], BF16), preferred_element_type=F32)

        def emit(i, j, y):
            blk = (pl.ds(i * R, R), pl.ds(j * 128, 128))
            res = xv[blk].astype(F32).reshape(R // 8, 8, 128) + bias_ref[:, pl.ds(j * 128, 128)]
            xv[blk] = (res.reshape(R, 128) + y).astype(BF16)

        _combine(prod, emit, _ORDER)

    def rhs(blk):
        for q in range(0, G, 128):
            b = {(k, j): blk(k, j, q) for k in range(3) for j in range(3)}
            for p, terms in enumerate(_RHS):
                v = b[terms[0][1:]]
                for sign, k, j in terms[1:]:
                    v = v + b[k, j] if sign > 0 else v - b[k, j]
                wc[p, pl.ds(q // 2, 64), :] = pltpu.bitcast(v.astype(BF16), U32)

    def prepare(t, ws):
        for cp in w1_copy(ws):
            cp.wait()
        rhs(lambda k, j, q: stage(ws)[pl.ds((j * G + q) // C * C + k * 128, 128),
                                      pl.ds((j * G + q) % C, 128)].astype(F32))
        x_head(0, tab[XS, t]).wait()
        for q in range(0, R, LNR):
            normalise(tab[XS, t], 0, q, ring[0])

    def lookup(t):
        return ([tab[XS, t + u] for u in range(U + 1)], [tab[HS, t + u] for u in range(U)],
                [tab[BUSY, t + u] for u in range(U)], tab[MORE, t + U - 1])

    def phase1(it, carry):
        t0 = it * U
        xs, hs, busy, more = carry
        x_rest(0, xs[0]).wait()
        for u in range(1, U):
            x_full(0, xs[u]).wait()
        pl.when(more > 0)(lambda: x_head(0, xs[U]).wait())
        xs = xs[:U] + [jnp.where(more > 0, xs[U], xs[0])]
        for u in range(U):
            pl.when(busy[u] > 0)(lambda: h_write(0, hs[u]).wait())
        for u in range(U):
            t = t0 + U * LX + u
            pl.when(tab[AHEAD, t0 + u] > 0)(lambda: fetch(tab[BLK, t], tab[XS, t], u == 0))
        zero = pl.multiple_of((it >> 20) * 8, 8)

        def piece(n):
            c, q = divmod(n, R // LNR)
            u, r = divmod((c + 1) * M, TB)
            dst = ring[(c + 1) % 2]
            normalise(xs[u], r, q * LNR, dst)
            pin_ref[n] = dst[pl.ds(zero, 8), pl.ds(0, 128)]

        todo = [functools.partial(piece, n) for n in range(U * TB // (2 * LNR))]
        for _ in range(_LEAD):
            todo.pop(0)()
        for c in range(U * TB // M):
            u, r = divmod(c * M, TB)
            expand(ring[c % 2], hslot(hs[u]).at[pl.ds(r // 2, R)], todo)
            left = (U * TB - (c + 1) * M) // (2 * LNR)
            assert left - R // LNR <= len(todo) <= left
            if r + M == TB:
                pl.when(tab[PUT, t0 + u] >= 0)(lambda: h_write(tab[PUT, t0 + u], hs[u]).start())
        return lookup(t0 + U)

    def rescale():
        w2_copy.wait()
        w2 = stage(S)
        row = lambda v: jnp.concatenate([v[k:k + 1, :] for k in range(D // 128)], axis=1)
        b = jnp.broadcast_to(row(b_ref[...].astype(F32)), (16, D)).astype(BF16)
        bias_ref[...] = jnp.dot(b, w2[...], preferred_element_type=F32)[:8]
        gx = jnp.sqrt(jnp.sum(acc_ref[...], axis=0, keepdims=True) * (1.0 / (_HS * _HS)) + 1e-6)
        nx = gx / (jnp.sum(gx, axis=-1, keepdims=True) * (1.0 / D) + 1e-6)
        scale = (row(g_ref[...].astype(F32)) * nx + 1.0) * (1.0 / _HS)
        col = functools.lru_cache(None)(lambda r: jnp.transpose(jnp.broadcast_to(scale[:, r:r + 128], (128, 128))))
        rhs(lambda k, j, q: w2[pl.ds(k * G + q, 128), pl.ds(j * 128, 128)].astype(F32) * col(k * G + q))
        for k in range(S, SX):
            x_full(k, k).start()

    nxt = lambda s, n: jnp.where(s == n - 1, 0, s + 1)

    def phase2(k, carry):
        xs, hs, ps, far = carry

        @pl.when(far > 0)
        def _():
            h_read(0, hs).wait()
            x_full(0, xs).wait()
        pl.when(k >= 2)(lambda: o_copy(0, ps).wait())
        i, j, n = tab[X_BLK, k], tab[H_BLK, k], tab[GET, k]
        pl.when(jnp.logical_and(i > 0, tab[SPLIT, k] == 0))(lambda: fetch(i, lax.rem(i, SX), False))
        pl.when(tab[SPLIT, k] > 0)(lambda: fetch(i, lax.rem(i, SX), True))

        @pl.when(k == at)
        def _():
            for cp in w1_copy(free_x):
                cp.start()
        half = TB // 2
        for r in range(0, TB, M):
            project(xs, hslot(hs), r)
            if (r + M) % half == 0:
                pl.when(k == 0)(lambda: h_read(0, 0, r + M - half, half).start())
                pl.when(k == nb - 1)(lambda: o_copy(nb - 1, (nb - 1) % SX, r + M - half, half).start())
        pl.when(jnp.logical_and(j > S, n >= 0))(lambda: h_read(n, lax.rem(j, S)).start())
        pl.when(k < nb - 1)(lambda: o_copy(k, xs).start())
        return nxt(xs, SX), nxt(hs, S), nxt(ps, SX), tab[FAR, k + 1]

    def shelve(back):
        for n in range(15 * G // 128):
            p, q = divmod(n, G // 128)
            r, c = divmod(n, D // 128)
            here = wc.at[p, pl.ds(q * 64, 64)]
            there = (pl.ds(free_h * (TB // 2) + r * 64, 64), pl.ds(c * 128, 128))
            if back:
                here[...] = hbuf[there]
            else:
                hbuf[there] = here[...]

    small = [pltpu.make_async_copy(src, dst, ssem.at[n]) for n, (src, dst) in enumerate(
        ((tab_hbm, tab), (dw_hbm, dw_ref), (g_hbm, g_ref), (b_hbm, b_ref)))]
    for cp in small + w1_copy(S):
        cp.start()
    acc_ref[...] = jnp.zeros_like(acc_ref)
    for cp in small:
        cp.wait()
    for t, (k, s) in enumerate(lead_in):
        fetch(k, s, t % U == 0)

    def sweep(rnd, carry):
        first = rnd == 0
        pick = lambda a, b: jnp.where(first, a, b)
        pl.when(rnd > 0)(functools.partial(shelve, False))
        prepare(pick(0, nb), pick(S, free_x))
        pl.when(first)(lambda: w2_copy.start())
        lax.fori_loop(pick(0, nb // U), pick(nb // U, nb // U + 1), phase1, lookup(pick(0, nb)))
        pl.when(first)(rescale)
        pl.when(rnd > 0)(functools.partial(shelve, True))
        return lax.fori_loop(pick(0, KR), pick(KR, nb), phase2, carry)

    lax.fori_loop(0, 2, sweep, (jnp.int32(0), jnp.int32(0), jnp.int32(S), jnp.int32(0)))
    for k in range(nb - 2, nb):
        o_copy(k, k % SX).wait()


@jax.jit
def pallas_standalone__modern_conv_block_slak__vision_kernel(
    x: jax.Array,
    dw: jax.Array,
    w1: jax.Array,
    w2: jax.Array,
    grn_g: jax.Array,
    grn_b: jax.Array,
):
    B, H, W, C = x.shape
    D = w1.shape[1]
    N = H * W
    assert B == 1 and dw.shape == (1, 1, C) and (C, D) == (384, 1536) and N % (U * TB) == 0
    nb = N // TB
    tab, parked, borrow = _plan(nb)
    hbm = pl.BlockSpec(memory_space=pl.ANY)
    out, _ = pl.pallas_call(
        functools.partial(_kernel, nb=nb, borrow=borrow,
                          lead_in=[(int(k), int(s)) for k, s in tab[[BLK, XS], :U * LX].T]),
        in_specs=[hbm] * 7,
        out_specs=[hbm, hbm],
        out_shape=[jax.ShapeDtypeStruct((N, C), BF16), jax.ShapeDtypeStruct((parked, TB // 2, D), U32)],
        scratch_shapes=[
            pltpu.VMEM(((S + 2) * TB + 64, C), BF16),
            pltpu.VMEM((S * TB // 2, D), U32),
            pltpu.VMEM((R // 2, 15 * 128), U32),
            pltpu.VMEM((R // 2, 15 * 128), U32),
            pltpu.VMEM((15, D // 6, 128), U32),
            pltpu.VMEM((8, D), F32),
            pltpu.VMEM((8, C), F32),
            pltpu.VMEM((U * TB // (2 * LNR), 8, 128), U32),
            pltpu.VMEM((1, C), dw.dtype),
            pltpu.VMEM((D // 128, 128), grn_g.dtype),
            pltpu.VMEM((D // 128, 128), grn_b.dtype),
            pltpu.SMEM(tab.shape, jnp.int32),
            pltpu.SemaphoreType.DMA((S + 2,)),
            pltpu.SemaphoreType.DMA((S + 2,)),
            pltpu.SemaphoreType.DMA((S,)),
            pltpu.SemaphoreType.DMA((S + 2,)),
            pltpu.SemaphoreType.DMA((D // C,)),
            pltpu.SemaphoreType.DMA((4,)),
        ],
        compiler_params=pltpu.CompilerParams(vmem_limit_bytes=int(127.9 * 2 ** 20), disable_bounds_checks=True),
        name="slak_block",
    )(tab, x.reshape(N, C).astype(BF16), dw.reshape(1, C), w1.astype(BF16), w2.astype(BF16),
      grn_g.reshape(D // 128, 128), grn_b.reshape(D // 128, 128))
    return out.reshape(B, H, W, C).astype(x.dtype)
```

```python
import functools
import math

import jax
import jax.experimental.pallas as pl
import jax.experimental.pallas.tpu as pltpu
import jax.numpy as jnp
import numpy as np
from jax import lax

F32, BF16, U32 = jnp.float32, jnp.bfloat16, jnp.uint32

_A = math.sqrt(2.0 / math.pi)
_K = (_A * 0.044715) ** (1.0 / 3.0)
_C0 = _A / _K
_HS = 2.0 * _K

R = 128
TB = 1024
U = 3
S = 32
NH = 12
LX = 2
KR = 103
PACE = (0.8, 4.5)
LNR = 16

_RHS = (
    ((+1, 2, 2), (+1, 1, 0), (-1, 2, 0)),
    ((+1, 1, 0),),
    ((+1, 2, 1), (+1, 2, 0), (+1, 0, 0)),
    ((+1, 0, 1),),
    ((+1, 2, 1), (+1, 1, 0)),
    ((+1, 0, 0),),
    ((+1, 2, 1),),
    ((+1, 1, 1), (-1, 2, 1), (-1, 1, 2)),
    ((+1, 1, 2),),
    ((+1, 1, 1), (+1, 1, 0), (+1, 0, 1)),
    ((+1, 2, 2),),
    ((+1, 2, 2), (+1, 0, 0)),
    ((+1, 1, 2), (+1, 0, 1)),
    ((+1, 2, 2), (+1, 0, 2), (-1, 0, 1)),
    ((+1, 1, 2), (+1, 0, 2), (-1, 0, 0)),
)
_PLAIN = {0: (1, 2), 2: (0, 2), 9: (0, 1), 14: (1, 0)}
_SHARED = {"p": (1, 4), "q": (9, "p"), "s": (11, 5), "t": (14, "s")}
_OUTS = {
    (0, 0): ((+1, 2), (+1, 5), (+1, 6), (+1, "p")),
    (0, 1): ((+1, 3), (+1, "q"), (-1, 6)),
    (1, 0): ((+1, 10), (+1, 1), (-1, 0), (-1, "s")),
    (1, 2): ((+1, 10), (+1, "t"), (-1, 8)),
    (0, 2): ((+1, 13), (+1, 3), (-1, 12), (+1, "t")),
    (1, 1): ((+1, 7), (+1, 12), (-1, 8), (+1, "q")),
}
_ORDER = (1, 4, 9, 6, 5, 2, 3, 11, 0, 10, 14, 8, 12, 13, 7)
_TILE_ORDER = (
    (5, 11, 8, 14, 10, 1, 0, 4, 6, 2, 9, 3, 12, 13, 7),
    (4, 1, 9, 6, 5, 2, 3, 11, 10, 0, 14, 8, 12, 13, 7),
    (1, 9, 4, 6, 3, 2, 5, 11, 0, 10, 14, 8, 12, 13, 7),
    (1, 4, 9, 6, 5, 2, 3, 11, 0, 10, 14, 8, 12, 13, 7),
)
_GATES = ((0, 5, 64), (0, 5, 96), (1, 4, 64), (1, 5, 0), (2, 3, 0), (2, 4, 32), (3, 5, 16), (3, 5, 120))
_LEAD = 2


def _lhs(a):
    @functools.lru_cache(None)
    def get(r):
        return {
            1: lambda: a(1, 1) + a(1, 2),
            3: lambda: a(0, 0) - a(0, 1),
            4: lambda: get(1) - a(0, 1),
            5: lambda: a(0, 0) - a(0, 2),
            6: lambda: get(4) - a(0, 2),
            7: lambda: a(1, 1) - a(0, 1),
            8: lambda: a(1, 0) - a(1, 1),
            10: lambda: get(11) + a(1, 2),
            11: lambda: get(5) - a(1, 0),
            12: lambda: a(1, 0) - a(0, 1),
            13: lambda: a(0, 0) - a(1, 0),
        }[r]()
    return get


def _combine(prod, emit, order):
    have, left = {}, dict(_OUTS)
    for r in order:
        have[r] = prod(r)
        for name, (u, v) in _SHARED.items():
            if name not in have and u in have and v in have:
                have[name] = have[u] - have[v]
        for out, terms in list(left.items()):
            if all(key in have for _, key in terms):
                age = list(have)
                terms = sorted(terms, key=lambda term: age.index(term[1]))
                sign, val = terms[0][0], have[terms[0][1]]
                for s, key in terms[1:]:
                    if s == sign:
                        val = val + have[key]
                    else:
                        sign, val = +1, (val - have[key] if sign > 0 else have[key] - val)
                assert sign > 0
                emit(*out, val)
                del left[out]


BLK, XS, HS, BUSY, PUT, AHEAD, MORE, H_BLK, GET, FAR, X_BLK, SPLIT = range(12)


def _plan(nb):
    redo = range(KR, KR + U)
    place = {k: n for n, k in enumerate(k for k in range(S, nb) if k not in redo)}
    keep, stream, order, n = list(range(NH, S)), list(range(S, nb)), [], nb - NH
    for t in range(n):
        due = (t + 1) * (S - NH) // n > t * (S - NH) // n
        order.append(keep.pop() if due else stream.pop())
    order += list(range(NH - 1, -1, -1))
    turn = {k: t // U for t, k in enumerate(order)}
    taken = {s: [(turn[s] - LX, turn[s])] for s in range(NH)}
    tab = np.zeros((12, nb + U * (LX + 2)), np.int32)
    dirty, c = [False] * S, 0
    for t, k in enumerate(order):
        if k < S:
            xs = hs = k
        else:
            lo, hi = t // U - LX, t // U
            xs = next(s for s in range(NH) if all(b < lo or a > hi for a, b in taken[s]))
            taken[xs].append((lo, hi))
            hs, c = c % NH, c + 1
        tab[:7, t] = k, xs, hs, dirty[hs], place.get(k, -1), t + U * LX < nb, t + 1 < nb
        dirty[hs] = k in place
    assert not any(dirty)
    for u, k in enumerate(redo):
        tab[:7, nb + u] = k, k % (S + 2), k % S, 0, -1, 0, u + 1 < U
    j, i, started = S, S + 2, dict.fromkeys(range(S), -1)
    for k in range(nb):
        clock = k + (U + 0.5 if k >= KR - U else 0)
        if j < nb and j - S <= k and (j - S < PACE[0] * clock + PACE[1] or j - k <= 2):
            tab[[H_BLK, GET], k] = j, place.get(j, -1)
            started[j] = k
            j += 1
        if i < j and i - (S + 2) <= k - 2:
            assert i > k and (i not in redo or k < KR)
            tab[[X_BLK, SPLIT], k] = i, i == KR
            i += 1
        tab[FAR, k] = k in place
    assert i == j == nb and started[S] == 0
    at = max(started[KR], KR - 11)
    held = lambda lo, n: [k % n for k in range(lo, nb) if started[k] < KR or k in redo]
    free_x = next(s for s in range(S + 1) if s not in held(at - 1, S + 2) and s + 1 not in held(at - 1, S + 2))
    free_h = next(s for s in range(S) if s not in held(KR - 1, S))
    return tab, len(place), (at, free_x, free_h)


def _kernel(tab_hbm, x_hbm, dw_hbm, w1_hbm, w2_hbm, g_hbm, b_hbm, o_hbm, h_hbm,
            xbuf, hbuf, ring0, ring1, wc, acc_ref, bias_ref, dwf_ref, pin_ref, dw_ref, g_ref, b_ref, tab,
            xsem, x0sem, hsem, osem, wsem, ssem, *, nb, lead_in, borrow):
    C, D = w1_hbm.shape
    G, M, SX = D // 3, 2 * R, S + 2
    ring = (ring0, ring1)
    at, free_x, free_h = borrow

    rows = lambda k, r, m: pl.ds(pl.multiple_of(k * TB + r, 16), m)
    xslot = lambda s: xbuf.at[pl.ds(pl.multiple_of(s * TB, TB), TB)]
    hslot = lambda s: hbuf.at[pl.ds(pl.multiple_of(s * (TB // 2), TB // 2), TB // 2)]
    x_copy = lambda k, s, r, m, sem: pltpu.make_async_copy(
        x_hbm.at[rows(k, r, m)], xslot(s).at[pl.ds(r, m)], sem.at[s])
    x_head = lambda k, s: x_copy(k, s, 0, M, x0sem)
    x_rest = lambda k, s: x_copy(k, s, M, TB - M, xsem)
    x_full = lambda k, s: x_copy(k, s, 0, TB, xsem)
    o_copy = lambda k, s, r=0, m=TB: pltpu.make_async_copy(
        xslot(s).at[pl.ds(r, m)], o_hbm.at[rows(k, r, m)], osem.at[s])
    h_write = lambda n, s: pltpu.make_async_copy(hslot(s), h_hbm.at[n], hsem.at[s])
    h_read = lambda n, s, r=0, m=TB: pltpu.make_async_copy(
        h_hbm.at[n, pl.ds(r // 2, m // 2)], hslot(s).at[pl.ds(r // 2, m // 2)], hsem.at[s])
    stage = lambda s: xbuf.at[pl.ds(pl.multiple_of(s * TB, TB), D)]
    w1_copy = lambda s: [pltpu.make_async_copy(w1_hbm.at[:, pl.ds(q * C, C)], stage(s).at[pl.ds(q * C, C)],
                                               wsem.at[q]) for q in range(D // C)]
    w2_copy = pltpu.make_async_copy(w2_hbm, stage(S), wsem.at[0])

    def fetch(k, s, split):
        for cp in (x_head(k, s), x_rest(k, s)) if split else (x_full(k, s),):
            cp.start()

    def layernorm(xs):
        ds, var = [], None
        for g, xv in enumerate(xs):
            y = xv * dwf_ref[...]
            d = y - jnp.sum(y, axis=-1, keepdims=True) * (1.0 / C)
            v = jnp.broadcast_to(jnp.sum(d * d, axis=-1, keepdims=True), (d.shape[0], 128))
            ds.append(d)
            var = v if var is None else jnp.where(lax.broadcasted_iota(jnp.int32, v.shape, 1) == g, v, var)
        inv = lax.rsqrt(var + 1e-5 * C) * (_K * math.sqrt(C))
        return [d * inv[:, g:g + 1] for g, d in enumerate(ds)]

    def normalise(s, r, q, dst):
        n = LNR // 8
        xs = [xslot(s)[pl.ds(r + i * R + q, LNR), :].astype(F32) for i in range(2)]
        normed = layernorm([v[8 * g:8 * g + 8] for v in xs for g in range(n)])
        halves = [jnp.concatenate(normed[i * n:(i + 1) * n], axis=0) for i in range(2)]
        blk = lambda i, k: halves[i][:, k * 128:(k + 1) * 128]
        lhs = _lhs(blk)
        for p in _ORDER:
            v = blk(*_PLAIN[p]) if p in _PLAIN else lhs(p)
            dst[pl.ds(q // 2, LNR // 2), pl.ds(p * 128, 128)] = pltpu.bitcast(v.astype(BF16), U32)

    def expand(src, hv, todo):
        for tile in range(G // 128):
            done = []

            def prod(p):
                return jnp.dot(pltpu.bitcast(src[:, pl.ds(p * 128, 128)], BF16),
                               pltpu.bitcast(wc[p, pl.ds(tile * 64, 64), :], BF16), preferred_element_type=F32)

            def emit(i, j, z):
                h = z * jnp.tanh(z * (z * z + _C0)) + z
                cols = pl.ds(j * G + tile * 128, 128)
                acc_ref[:, cols] += jnp.sum((h * h).reshape(R // 8, 8, 128), axis=0)
                hv[pl.ds(i * R // 2, R // 2), cols] = pltpu.bitcast(h.astype(BF16), U32)
                for gate in _GATES:
                    if gate[:2] == (tile, len(done)) and todo:
                        xbuf[pl.ds(SX * TB, 8), pl.ds(0, 128)] = z[gate[2]:gate[2] + 8].astype(BF16)
                        todo.pop(0)()
                done.append((i, j))

            _combine(prod, emit, _TILE_ORDER[tile])

    def project(s, hv, r):
        raw = lambda i, k: pltpu.bitcast(hv[pl.ds((r + i * R) // 2, R // 2), pl.ds(k * G, G)], BF16)
        lhs = _lhs(lambda i, k: raw(i, k).astype(F32))
        xv = xslot(s).at[pl.ds(r, M)]

        def prod(p):
            a = raw(*_PLAIN[p]) if p in _PLAIN else lhs(p).astype(BF16)
            return jnp.dot(a, pltpu.bitcast(wc[p], BF16), preferred_element_type=F32)

        def emit(i, j, y):
            blk = (pl.ds(i * R, R), pl.ds(j * 128, 128))
            res = xv[blk].astype(F32).reshape(R // 8, 8, 128) + bias_ref[:, pl.ds(j * 128, 128)]
            xv[blk] = (res.reshape(R, 128) + y).astype(BF16)

        _combine(prod, emit, _ORDER)

    def rhs(blk):
        for q in range(0, G, 128):
            b = {(k, j): blk(k, j, q) for k in range(3) for j in range(3)}
            for p, terms in enumerate(_RHS):
                v = b[terms[0][1:]]
                for sign, k, j in terms[1:]:
                    v = v + b[k, j] if sign > 0 else v - b[k, j]
                wc[p, pl.ds(q // 2, 64), :] = pltpu.bitcast(v.astype(BF16), U32)

    def prepare(t, ws):
        for cp in w1_copy(ws):
            cp.wait()
        rhs(lambda k, j, q: stage(ws)[pl.ds((j * G + q) // C * C + k * 128, 128),
                                      pl.ds((j * G + q) % C, 128)].astype(F32))
        x_head(0, tab[XS, t]).wait()
        for q in range(0, R, LNR):
            normalise(tab[XS, t], 0, q, ring[0])

    def lookup(t):
        return ([tab[XS, t + u] for u in range(U + 1)], [tab[HS, t + u] for u in range(U)],
                [tab[BUSY, t + u] for u in range(U)], tab[MORE, t + U - 1])

    def phase1(it, carry):
        t0 = it * U
        xs, hs, busy, more = carry
        x_rest(0, xs[0]).wait()
        for u in range(1, U):
            x_full(0, xs[u]).wait()
        pl.when(more > 0)(lambda: x_head(0, xs[U]).wait())
        xs = xs[:U] + [jnp.where(more > 0, xs[U], xs[0])]
        for u in range(U):
            pl.when(busy[u] > 0)(lambda: h_write(0, hs[u]).wait())
        for u in range(U):
            t = t0 + U * LX + u
            pl.when(tab[AHEAD, t0 + u] > 0)(lambda: fetch(tab[BLK, t], tab[XS, t], u == 0))
        zero = pl.multiple_of((it >> 20) * 8, 8)

        def piece(n):
            c, q = divmod(n, R // LNR)
            u, r = divmod((c + 1) * M, TB)
            dst = ring[(c + 1) % 2]
            normalise(xs[u], r, q * LNR, dst)
            pin_ref[n] = dst[pl.ds(zero, 8), pl.ds(0, 128)]

        todo = [functools.partial(piece, n) for n in range(U * TB // (2 * LNR))]
        for _ in range(_LEAD):
            todo.pop(0)()
        for c in range(U * TB // M):
            u, r = divmod(c * M, TB)
            expand(ring[c % 2], hslot(hs[u]).at[pl.ds(r // 2, R)], todo)
            left = (U * TB - (c + 1) * M) // (2 * LNR)
            assert left - R // LNR <= len(todo) <= left
            if r + M == TB:
                pl.when(tab[PUT, t0 + u] >= 0)(lambda: h_write(tab[PUT, t0 + u], hs[u]).start())
        return lookup(t0 + U)

    def rescale():
        w2_copy.wait()
        w2 = stage(S)
        row = lambda v: jnp.concatenate([v[k:k + 1, :] for k in range(D // 128)], axis=1)
        b = jnp.broadcast_to(row(b_ref[...].astype(F32)), (16, D)).astype(BF16)
        bias_ref[...] = jnp.dot(b, w2[...], preferred_element_type=F32)[:8]
        gx = jnp.sqrt(jnp.sum(acc_ref[...], axis=0, keepdims=True) * (1.0 / (_HS * _HS)) + 1e-6)
        nx = gx / (jnp.sum(gx, axis=-1, keepdims=True) * (1.0 / D) + 1e-6)
        scale = (row(g_ref[...].astype(F32)) * nx + 1.0) * (1.0 / _HS)
        col = functools.lru_cache(None)(lambda r: jnp.transpose(jnp.broadcast_to(scale[:, r:r + 128], (128, 128))))
        rhs(lambda k, j, q: w2[pl.ds(k * G + q, 128), pl.ds(j * 128, 128)].astype(F32) * col(k * G + q))
        for k in range(S, SX):
            x_full(k, k).start()

    nxt = lambda s, n: jnp.where(s == n - 1, 0, s + 1)

    def phase2(k, carry):
        xs, hs, ps, far = carry

        @pl.when(far > 0)
        def _():
            h_read(0, hs).wait()
            x_full(0, xs).wait()
        pl.when(k >= 2)(lambda: o_copy(0, ps).wait())
        i, j, n = tab[X_BLK, k], tab[H_BLK, k], tab[GET, k]
        pl.when(jnp.logical_and(i > 0, tab[SPLIT, k] == 0))(lambda: fetch(i, lax.rem(i, SX), False))
        pl.when(tab[SPLIT, k] > 0)(lambda: fetch(i, lax.rem(i, SX), True))

        @pl.when(k == at)
        def _():
            for cp in w1_copy(free_x):
                cp.start()
        half = TB // 2
        for r in range(0, TB, M):
            project(xs, hslot(hs), r)
            if (r + M) % half == 0:
                pl.when(k == 0)(lambda: h_read(0, 0, r + M - half, half).start())
                pl.when(k == nb - 1)(lambda: o_copy(nb - 1, (nb - 1) % SX, r + M - half, half).start())
        pl.when(jnp.logical_and(j > S, n >= 0))(lambda: h_read(n, lax.rem(j, S)).start())
        pl.when(k < nb - 1)(lambda: o_copy(k, xs).start())
        return nxt(xs, SX), nxt(hs, S), nxt(ps, SX), tab[FAR, k + 1]

    def shelve(back):
        for n in range(15 * G // 128):
            p, q = divmod(n, G // 128)
            r, c = divmod(n, D // 128)
            here = wc.at[p, pl.ds(q * 64, 64)]
            there = (pl.ds(free_h * (TB // 2) + r * 64, 64), pl.ds(c * 128, 128))
            if back:
                here[...] = hbuf[there]
            else:
                hbuf[there] = here[...]

    small = [pltpu.make_async_copy(src, dst, ssem.at[n]) for n, (src, dst) in enumerate(
        ((tab_hbm, tab), (dw_hbm, dw_ref), (g_hbm, g_ref), (b_hbm, b_ref)))]
    for cp in small + w1_copy(S):
        cp.start()
    acc_ref[...] = jnp.zeros_like(acc_ref)
    for cp in small:
        cp.wait()
    for t, (k, s) in enumerate(lead_in):
        fetch(k, s, t % U == 0)
    dwf_ref[...] = jnp.broadcast_to(dw_ref[...].astype(F32), (8, C))

    def sweep(rnd, carry):
        first = rnd == 0
        pick = lambda a, b: jnp.where(first, a, b)
        pl.when(rnd > 0)(functools.partial(shelve, False))
        prepare(pick(0, nb), pick(S, free_x))
        pl.when(first)(lambda: w2_copy.start())
        lax.fori_loop(pick(0, nb // U), pick(nb // U, nb // U + 1), phase1, lookup(pick(0, nb)))
        pl.when(first)(rescale)
        pl.when(rnd > 0)(functools.partial(shelve, True))
        return lax.fori_loop(pick(0, KR), pick(KR, nb), phase2, carry)

    lax.fori_loop(0, 2, sweep, (jnp.int32(0), jnp.int32(0), jnp.int32(S), jnp.int32(0)))
    for k in range(nb - 2, nb):
        o_copy(k, k % SX).wait()


@jax.jit
def pallas_standalone__modern_conv_block_slak__vision_kernel(
    x: jax.Array,
    dw: jax.Array,
    w1: jax.Array,
    w2: jax.Array,
    grn_g: jax.Array,
    grn_b: jax.Array,
):
    B, H, W, C = x.shape
    D = w1.shape[1]
    N = H * W
    assert B == 1 and dw.shape == (1, 1, C) and (C, D) == (384, 1536) and N % (U * TB) == 0
    nb = N // TB
    tab, parked, borrow = _plan(nb)
    hbm = pl.BlockSpec(memory_space=pl.ANY)
    out, _ = pl.pallas_call(
        functools.partial(_kernel, nb=nb, borrow=borrow,
                          lead_in=[(int(k), int(s)) for k, s in tab[[BLK, XS], :U * LX].T]),
        in_specs=[hbm] * 7,
        out_specs=[hbm, hbm],
        out_shape=[jax.ShapeDtypeStruct((N, C), BF16), jax.ShapeDtypeStruct((parked, TB // 2, D), U32)],
        scratch_shapes=[
            pltpu.VMEM(((S + 2) * TB + 64, C), BF16),
            pltpu.VMEM((S * TB // 2, D), U32),
            pltpu.VMEM((R // 2, 15 * 128), U32),
            pltpu.VMEM((R // 2, 15 * 128), U32),
            pltpu.VMEM((15, D // 6, 128), U32),
            pltpu.VMEM((8, D), F32),
            pltpu.VMEM((8, C), F32),
            pltpu.VMEM((8, C), F32),
            pltpu.VMEM((U * TB // (2 * LNR), 8, 128), U32),
            pltpu.VMEM((1, C), dw.dtype),
            pltpu.VMEM((D // 128, 128), grn_g.dtype),
            pltpu.VMEM((D // 128, 128), grn_b.dtype),
            pltpu.SMEM(tab.shape, jnp.int32),
            pltpu.SemaphoreType.DMA((S + 2,)),
            pltpu.SemaphoreType.DMA((S + 2,)),
            pltpu.SemaphoreType.DMA((S,)),
            pltpu.SemaphoreType.DMA((S + 2,)),
            pltpu.SemaphoreType.DMA((D // C,)),
            pltpu.SemaphoreType.DMA((4,)),
        ],
        compiler_params=pltpu.CompilerParams(vmem_limit_bytes=int(127.9 * 2 ** 20), disable_bounds_checks=True),
        name="slak_block",
    )(tab, x.reshape(N, C).astype(BF16), dw.reshape(1, C), w1.astype(BF16), w2.astype(BF16),
      grn_g.reshape(D // 128, 128), grn_b.reshape(D // 128, 128))
    return out.reshape(B, H, W, C).astype(x.dtype)
```
